```python
import jax
import jax.numpy as jnp

def _softmax(x, axis=-1):
    return jax.nn.softmax(x, axis=axis)

def _gelu(x):
    return jax.nn.gelu(x, approximate=True)

def _silu(x):
    return jax.nn.silu(x)

def _sigmoid(x):
    return jax.nn.sigmoid(x)

def _layernorm(x, axis=-1, eps=1e-05):
    m = jnp.mean(x, axis=axis, keepdims=True)
    v = jnp.var(x, axis=axis, keepdims=True)
    return (x - m) / jnp.sqrt(v + eps)

def _scatter_add(tgt, idx, src, axis=0):
    return tgt.at[idx].add(src)

def _segment_sum(src, seg, n):
    return jax.ops.segment_sum(src, seg, n)

class _Rng:

    def __init__(self, key):
        self._k = key

    def _next(self):
        self._k, sub = jax.random.split(self._k)
        return sub

    def normal(self, shape):
        return jax.random.normal(self._next(), shape, dtype=jnp.bfloat16)

    def randint(self, lo, hi, shape):
        return jax.random.randint(self._next(), shape, lo, hi, dtype=jnp.int32)

    def uniform(self, shape, lo=0.0, hi=1.0):
        return jax.random.uniform(self._next(), shape, jnp.bfloat16, lo, hi)

    def permutation(self, n):
        return jax.random.permutation(self._next(), n)
kernel_name = 'adaLN_cond__spectral_gfnet__mixer_token_mlp__prompt'

def setup_inputs():
    _rng = _Rng(jax.random.key(int.from_bytes(__import__("os").urandom(4), "little")))
    _w = lambda a: (lambda t: t.astype(jnp.bfloat16) if jnp.issubdtype(t.dtype, jnp.floating) else t)(jnp.asarray(a))

    def _A_setup():
        B, S, D = (1, 2048, 576)
        Df = D // 2 + 1
        return {'x': _w((lambda *s: _rng.normal(s) * 0.05)(B, S, D)), 'w_r': _w((lambda *s: _rng.normal(s) * 0.05)(S, Df) * 0.02), 'w_i': _w((lambda *s: _rng.normal(s) * 0.05)(S, Df) * 0.02)}
    _A_in = _A_setup()

    def _B_setup():
        B, S, D, F = (1, 2048, 576, 4608)
        return {'x': _w((lambda *s: _rng.normal(s) * 0.05)(B, S, D)), 'w1': _w((lambda *s: _rng.normal(s) * 0.05)(S, F) * S ** (-0.5)), 'b1': _w((lambda *s: _rng.normal(s) * 0.05)(F) * 0.02), 'w2': _w((lambda *s: _rng.normal(s) * 0.05)(F, S) * F ** (-0.5)), 'b2': _w((lambda *s: _rng.normal(s) * 0.05)(S) * 0.02)}
    _B_in = _B_setup()
    return {'A_x': _A_in['x'], 'A_w_r': _A_in['w_r'], 'A_w_i': _A_in['w_i'], 'B_x': _B_in['x'], 'B_w1': _B_in['w1'], 'B_b1': _B_in['b1'], 'B_w2': _B_in['w2'], 'B_b2': _B_in['b2'], 'c': _w((lambda *s: _rng.normal(s) * 0.05)(1, 576)), 'w_mod': _w((lambda *s: _rng.normal(s) * 0.05)(576, 6 * 576) * 576 ** (-0.5))}

def reference(A_x, A_w_r, A_w_i, B_x, B_w1, B_b1, B_w2, B_b2, c, w_mod):

    def _A_ref(x, w_r, w_i):
        B, S, D = x.shape
        X = (lambda x, axes=(-2, -1): jnp.fft.rfft2(x.astype(jnp.float32), axes=axes))(x, axes=(-2, -1))
        W = w_r + 1j * w_i
        X = X * W
        y = (lambda x, s, axes=(-2, -1): jnp.fft.irfft2(x, s=s, axes=axes).astype(jnp.bfloat16))(X, (S, D), axes=(-2, -1))
        return y

    def _B_ref(x, w1, b1, w2, b2):
        B, S, D = x.shape
        h = _layernorm(x, axis=-1)
        u = jnp.einsum('bsd,sf->bdf', h, w1) + b1
        u = _gelu(u)
        y = jnp.einsum('bdf,fs->bds', u, w2) + b2
        return (lambda x, *d: x.transpose(*d))(y, 0, 2, 1)
    x = A_x
    mod = (_silu(c) @ w_mod).reshape(c.shape[0], 6, 1, -1)
    sa, ca, ga, sb, cb, gb = (mod[:, 0].copy(), mod[:, 1].copy(), mod[:, 2].copy(), mod[:, 3].copy(), mod[:, 4].copy(), mod[:, 5].copy())
    h = _layernorm(x, axis=-1) * (1 + ca) + sa
    x = x + ga * _A_ref(h, A_w_r, A_w_i)
    h = _layernorm(x, axis=-1) * (1 + cb) + sb
    x = x + gb * _B_ref(h, B_w1, B_b1, B_w2, B_b2)
    return x
```

```python
import numpy as np

import jax
import jax.numpy as jnp
import jax.experimental.pallas as pl
import jax.experimental.pallas.tpu as pltpu

S, D, F = 2048, 576, 4608
DF = D // 2 + 1
L = 128
NT = S // L
R = 304
EPS = 1e-5
f32, bf16, u32 = jnp.float32, jnp.bfloat16, jnp.uint32

_ORDER = (1, 10, 8, 17, 2, 11, 7, 16, 3, 12, 6, 15, 4, 13, 5, 14, 0, 9)
_S3 = float(np.sqrt(3.0) / 2)
_C1, _C2, _C4 = (float(np.cos(2 * np.pi * k / 9)) for k in (1, 2, 4))
_S1, _S2, _S4 = (float(np.sin(2 * np.pi * k / 9)) for k in (1, 2, 4))


def _channel_dft_matrices():
    dp = np.arange(64)
    fw = np.zeros((5, 128, 128))
    iv = np.zeros((5, 128, 128))
    for g in range(4):
        r = g + 1
        bs = _S3 if r == 3 else 1.0
        for q in range(4):
            rho = _ORDER[4 * g + q]
            sig = 1.0 if rho % 9 == r else -1.0
            for m in range(16):
                phi = 2 * np.pi * dp * (18 * m + rho) / D
                row = 16 * q + m
                fw[g, row, :64] = np.cos(phi)
                fw[g, row, 64:] = -sig * bs * np.sin(phi)
                fw[g, 64 + row, :64] = -np.sin(phi)
                fw[g, 64 + row, 64:] = -sig * bs * np.cos(phi)
                c = 2.0 / (D * S)
                iv[g, :64, row] = c * np.cos(phi)
                iv[g, :64, 64 + row] = -c * np.sin(phi)
                iv[g, 64:, row] = bs * sig * c * np.sin(phi)
                iv[g, 64:, 64 + row] = bs * sig * c * np.cos(phi)
    for q in range(2):
        for m in range(16):
            kd = 18 * m + _ORDER[16 + q]
            phi = 2 * np.pi * dp * kd / D
            row = 16 * q + m
            c = (1.0 if kd == 0 else 2.0) / (D * S)
            fw[4, row, :64] = np.cos(phi)
            fw[4, 48 + row, :64] = -np.sin(phi)
            iv[4, :64, row] = c * np.cos(phi)
            iv[4, :64, 48 + row] = -c * np.sin(phi)
    fw[4, 32, :64] = np.cos(np.pi * dp)
    iv[4, :64, 32] = np.cos(np.pi * dp) / (D * S)
    return np.concatenate([fw, iv], 0).astype(np.float32)


_DMAT = _channel_dft_matrices()


def _radix9(h0, p1, p2, p3, p4, m1, m2, q, m4):
    e = p1 + p2 + p4
    f = h0 + p3
    base = h0 - 0.5 * p3
    a, b = p1 - p4, p2 - p4
    r1, r2 = _C1 * a + _C2 * b, _C2 * a + _C4 * b
    u, v = m1 + m2, m2 + m4
    i1, i2 = _S1 * u + _S4 * v, _S2 * u - _S1 * v
    return ((f + e, base + r1, base + r2, f - 0.5 * e, base - (r1 + r2)),
            (i1 + q, i2 - q, m1 - m2 + m4, (i2 - i1) + q))


def _radix4(x0, x1, x2, x3, inverse):
    t0 = (x0[0] + x2[0], x0[1] + x2[1])
    t1 = (x0[0] - x2[0], x0[1] - x2[1])
    return _radix4_tail(t0, t1, x1, x3, inverse)


def _radix4_tail(t0, t1, x1, x3, inverse):
    t2 = (x1[0] + x3[0], x1[1] + x3[1])
    t3 = (x1[0] - x3[0], x1[1] - x3[1])
    ya = (t1[0] + t3[1], t1[1] - t3[0])
    yb = (t1[0] - t3[1], t1[1] + t3[0])
    if inverse:
        ya, yb = yb, ya
    return [(t0[0] + t2[0], t0[1] + t2[1]), ya, (t0[0] - t2[0], t0[1] - t2[1]), yb]


def _twiddle16(z, n, inverse):
    if n == 0:
        return z
    c = float(np.cos(2 * np.pi * n / 16))
    s = float(np.sin(2 * np.pi * n / 16)) * (-1.0 if inverse else 1.0)
    re, im = z
    if n % 4 == 2:
        if c * s > 0:
            return ((re + im) * c, (im - re) * c)
        return ((re - im) * c, (im + re) * c)
    return (re * c + im * s, im * c - re * s)


def _fft16(x, inverse):
    a = [_radix4(x[a0], x[4 + a0], x[8 + a0], x[12 + a0], inverse) for a0 in range(4)]
    out = [None] * 16
    for k0 in range(4):
        x0, x1, x3 = a[0][k0], _twiddle16(a[1][k0], k0, inverse), _twiddle16(a[3][k0], 3 * k0, inverse)
        if k0 == 2:
            x2 = a[2][k0]
            ta, tb = (x0[0] + x2[1], x0[1] - x2[0]), (x0[0] - x2[1], x0[1] + x2[0])
            t0, t1 = (tb, ta) if inverse else (ta, tb)
            y = _radix4_tail(t0, t1, x1, x3, inverse)
        else:
            y = _radix4(x0, x1, _twiddle16(a[2][k0], 2 * k0, inverse), x3, inverse)
        for k1 in range(4):
            out[k0 + 4 * k1] = y[k1]
    return out


def _dot(a, b):
    return jnp.dot(a, b, preferred_element_type=f32)


def _dot_nt(a, b):
    return jax.lax.dot_general(a, b, (((1,), (1,)), ((), ())), preferred_element_type=f32)


def _center_rstd(x):
    xc = x - jnp.sum(x, axis=0, keepdims=True) * (1.0 / D)
    var = jnp.sum(xc * xc, axis=0, keepdims=True) * (1.0 / D)
    return xc, jax.lax.rsqrt(var + EPS)


def _gelu(x):
    k = float(np.sqrt(2 / np.pi))
    t = jnp.tanh(x * (x * x * (k * 0.044715) + k))
    hx = 0.5 * x
    return hx * t + hx


def _badd(x, y):
    return (x.astype(f32) + y.astype(f32)).astype(bf16)


def _bsub(x, y):
    return (x.astype(f32) - y.astype(f32)).astype(bf16)


def _lhs_operands(a11, a12, a21, a22):
    return (a11 + a22, a21 + a22, a11, a22, a11 + a12, a21 - a11, a12 - a22)


def _strassen(lhs, b11, b12, b21, b22, emit):
    m3 = _dot(lhs(2), _bsub(b12(), b22()))
    m5 = _dot(lhs(4), b22())
    emit(0, 1, m3 + m5)
    m2 = _dot(lhs(1), b11())
    m4 = _dot(lhs(3), _bsub(b21(), b11()))
    emit(1, 0, m2 + m4)
    m1 = _dot(lhs(0), _badd(b11(), b22()))
    m7 = _dot(lhs(6), _badd(b21(), b22()))
    emit(0, 0, (m4 - m5) + m1 + m7)
    m6 = _dot(lhs(5), _badd(b11(), b12()))
    emit(1, 1, (m3 - m2) + m1 + m6)


XC = 4
FC = 256
SC = 256
N1 = F // 2 // FC
N2 = S // 2 // SC
HD = D // 2


def _kernel(xT_hbm, wr_hbm, wi_hbm, w1_hbm, b1_hbm, w2_hbm, b2_hbm, c_hbm, wm_hbm, dm_hbm, o_hbm,
            x_v, wr_v, wi_v, w1_v, b1_v, w2_v, b2_v, c_v, wm_v, dm_v,
            b1_f, b2_f, mod_v, t_v, wp_v, sp_v, g_v, v_v, x1_v, a1_v, a2_v, o_v,
            sem, sem_x, sem_w1, sem_o):
    def lanes(i, n=L):
        return pl.ds(pl.multiple_of(i * n, n), n)

    cp_c = pltpu.make_async_copy(c_hbm, c_v, sem.at[0])
    cp_wma = pltpu.make_async_copy(wm_hbm.at[:, 0:2 * D], wm_v.at[:, 0:2 * D], sem.at[1])
    cp_dm = pltpu.make_async_copy(dm_hbm, dm_v, sem.at[2])
    cp_wr = pltpu.make_async_copy(wr_hbm, wr_v, sem.at[3])
    cp_wi = pltpu.make_async_copy(wi_hbm, wi_v, sem.at[4])
    cp_wmb = pltpu.make_async_copy(wm_hbm.at[:, 2 * D:6 * D], wm_v.at[:, 2 * D:6 * D], sem.at[5])
    cp_b1 = pltpu.make_async_copy(b1_hbm, b1_v, sem.at[6])
    cp_b2 = pltpu.make_async_copy(b2_hbm, b2_v, sem.at[7])
    cp_w2 = pltpu.make_async_copy(w2_hbm, w2_v, sem.at[8])

    def cp_x(i):
        return pltpu.make_async_copy(xT_hbm.at[:, lanes(i, S // XC)], x_v.at[:, lanes(i, S // XC)], sem_x.at[i])

    def cp_w1(j, h):
        cols = lanes(j + h * N1, FC)
        return pltpu.make_async_copy(w1_hbm.at[:, cols], w1_v.at[:, cols], sem_w1.at[j + h * N1])

    def cp_o(j, h):
        cols = lanes(j + h * N2, SC)
        return pltpu.make_async_copy(o_v.at[:, cols], o_hbm.at[:, cols], sem_o.at[j + h * N2])

    cp_c.start()
    cp_wma.start()
    cp_dm.start()
    for i in range(XC):
        cp_x(i).start()

    row = jax.lax.broadcasted_iota(jnp.int32, (L, L), 0)
    lane = jax.lax.broadcasted_iota(jnp.int32, (L, L), 1)
    ang = ((row * (8 * (lane & 15) + (lane >> 4))) & 127).astype(f32) * float(2 * np.pi / L)
    step = row.astype(f32) * float(2 * np.pi / S)
    ec, es = jnp.cos(step), jnp.sin(step)

    def t_body(k1, cs):
        c, s = cs
        t_v[k1, 0] = c.astype(bf16)
        t_v[k1, 1] = (c - s).astype(bf16)
        t_v[k1, 2] = (-s - c).astype(bf16)
        c, s = pltpu.roll(c, 1, 1), pltpu.roll(s, 1, 1)
        return c * ec - s * es, s * ec + c * es

    jax.lax.fori_loop(0, NT, t_body, (jnp.cos(ang), jnp.sin(ang)))

    cp_c.wait()
    cf = c_v[...].astype(f32)
    sc = jnp.broadcast_to(cf * jax.nn.sigmoid(cf), (16, D)).astype(bf16)

    def modulation(t0, t1):
        m = _dot(sc, wm_v[:, t0 * L:t1 * L])
        for t in range(t0, t1):
            col = jnp.broadcast_to(m[0:1, (t - t0) * L:(t - t0 + 1) * L], (L, L)).T
            idx = t * L + jax.lax.broadcasted_iota(jnp.int32, (L, L), 0)
            is_scale = ((idx >= D) & (idx < 2 * D)) | ((idx >= 4 * D) & (idx < 5 * D))
            mod_v[t * L:(t + 1) * L, :] = jnp.where(is_scale, col + 1.0, col)

    cp_wma.wait()
    modulation(0, 2 * D // L)
    cp_wr.start()
    cp_wi.start()

    cp_dm.wait()

    def fwd_body(i, carry):
        cp_x(i).wait()
        for t in range(NT // XC):
            a = i * (NT // XC) + t
            xc, rs = _center_rstd(x_v[:, lanes(a)].astype(f32))
            h = xc * rs * mod_v[D:2 * D, :] + mod_v[0:D, :]
            hb = [h[64 * j:64 * j + 64] for j in range(9)]
            p = [hb[j] + hb[9 - j] for j in range(1, 5)]
            m = [hb[j] - hb[9 - j] for j in range(1, 5)]
            ev, od = _radix9(hb[0], p[0], p[1], p[2], p[3], m[0], m[1], _S3 * m[2], m[3])
            for g in range(4):
                o = _dot(dm_v[g], jnp.concatenate([ev[g + 1], od[g]], axis=0).astype(bf16))
                sp_v[a, 0, 64 * g:64 * g + 64, :] = o[0:64]
                sp_v[a, 1, 64 * g:64 * g + 64, :] = o[64:128]
            o = _dot(dm_v[4, 0:80, 0:64], ev[0].astype(bf16))
            sp_v[a, 0, 256:R, :] = o[0:48]
            sp_v[a, 1, 256:288, :] = o[48:80]
            sp_v[a, 1, 288:R, :] = jnp.zeros((16, L), f32)
        return carry

    jax.lax.fori_loop(0, XC, fwd_body, 0)
    cp_wmb.start()
    cp_b1.start()
    cp_b2.start()
    cp_w1(0, 0).start()
    cp_w1(0, 1).start()

    def r16_fwd(p, carry):
        rows = lanes(p, 16)
        y = _fft16([(sp_v[a, 0, rows, :], sp_v[a, 1, rows, :]) for a in range(NT)], False)
        for k in range(NT):
            g_v[k, 0, rows, :] = (y[k][0] + y[k][1]).astype(bf16)
            g_v[k, 1, rows, :] = y[k][1].astype(bf16)
            g_v[k, 2, rows, :] = y[k][0].astype(bf16)
        return carry

    jax.lax.fori_loop(0, R // 16, r16_fwd, 0)

    KU = 4

    def mxu_fwd(i, carry):
        for t in range(KU):
            k = i * KU + t
            p1 = _dot(g_v[k, 0], t_v[k, 0])
            sp_v[k, 0] = p1 - _dot(g_v[k, 1], t_v[k, 1])
            sp_v[k, 1] = p1 + _dot(g_v[k, 2], t_v[k, 2])
        return carry

    jax.lax.fori_loop(0, NT // KU, mxu_fwd, 0)

    lane8 = jax.lax.broadcasted_iota(jnp.int32, (8, L), 1)

    def permute(tiles, z, rows):
        rot = [tiles[0]] + [pltpu.roll(tiles[j], j, 1) for j in range(1, NT)]
        cur = [rot[-i % NT] for i in range(NT)]
        for b in range(4):
            mask = ((lane8 >> b) & 1) == 1
            cur = [jnp.where(mask, cur[(i - (1 << b)) % NT], cur[i]) for i in range(NT)]
        for k in range(NT):
            wp_v[k, z, rows, :] = cur[k]

    cp_wr.wait()
    cp_wi.wait()

    def wp_body(p, carry):
        for z, w_v in enumerate((wr_v, wi_v)):
            permute([pltpu.bitcast(w_v[lanes(p, 16), j * L:(j + 1) * L], u32) for j in range(NT)], z, lanes(p, 8))
        return carry

    jax.lax.fori_loop(0, (DF - 1) // 16, wp_body, 0)
    for z, w_v in enumerate((wr_v, wi_v)):
        nyq = w_v[DF - 1:DF, :].astype(f32)
        permute([pltpu.bitcast(jnp.broadcast_to(nyq[:, j * L:(j + 1) * L], (8, L)), u32) for j in range(NT)],
                z, slice(144, 152))
    for j in range(1, N1):
        cp_w1(j, 0).start()
        cp_w1(j, 1).start()

    def filt(k, z):
        blocks = []
        for rho in _ORDER:
            w = wp_v[k, z, pl.ds(rho // 2, 16, stride=9), :]
            blocks.append(pltpu.bitcast((w & u32(0xFFFF0000)) if rho % 2 else (w << 16), f32))
        nyq = pltpu.bitcast(wp_v[k, z, 144:152, :], f32)
        return jnp.concatenate(blocks + [nyq, nyq], axis=0)

    def mxu_inv(i, carry):
        for t in range(KU):
            k = i * KU + t
            xr, xi = sp_v[k, 0], sp_v[k, 1]
            wr, wi = filt(k, 0), filt(k, 1)
            yr, yi = xr * wr - xi * wi, xr * wi + xi * wr
            q1 = _dot_nt((yr + yi).astype(bf16), t_v[k, 0])
            sp_v[k, 0] = q1 + _dot_nt(yi.astype(bf16), t_v[k, 2])
            sp_v[k, 1] = q1 - _dot_nt(yr.astype(bf16), t_v[k, 1])
        return carry

    jax.lax.fori_loop(0, NT // KU, mxu_inv, 0)

    def r16_inv(p, carry):
        rows = lanes(p, 16)
        y = _fft16([(sp_v[k, 0, rows, :], sp_v[k, 1, rows, :]) for k in range(NT)], True)
        for a in range(NT):
            v_v[a, 0, rows, :] = y[a][0].astype(bf16)
            v_v[a, 1, rows, :] = y[a][1].astype(bf16)
        return carry

    jax.lax.fori_loop(0, R // 16, r16_inv, 0)

    cp_wmb.wait()
    modulation(2 * D // L, 6 * D // L)
    cp_b1.wait()
    cp_b2.wait()
    b1_f[...] = b1_v[...].astype(f32)
    b2_f[...] = b2_v[...].astype(f32)

    def token_tile(a):
        al, be = [], []
        for g in range(4):
            rhs = jnp.concatenate([v_v[a, 0, 64 * g:64 * g + 64, :], v_v[a, 1, 64 * g:64 * g + 64, :]], axis=0)
            o = _dot(dm_v[5 + g], rhs)
            al.append(o[0:64])
            be.append(o[64:128])
        rhs = jnp.concatenate([v_v[a, 0, 256:R, :], v_v[a, 1, 256:288, :]], axis=0)
        w0 = _dot(dm_v[9, 0:64, 0:80], rhs)
        ev, od = _radix9(w0, al[0], al[1], al[2], al[3], be[0], be[1], be[2], be[3])
        od = (od[0], od[1], _S3 * od[2], od[3])
        y = jnp.concatenate([ev[0]] + [ev[j + 1] - od[j] for j in range(4)]
                            + [ev[j + 1] + od[j] for j in (3, 2, 1, 0)], axis=0)
        x1 = x_v[:, lanes(a)].astype(f32) + mod_v[2 * D:3 * D, :] * y
        x1_v[:, lanes(a)] = x1
        xc, rs = _center_rstd(x1)
        xc, rs = _center_rstd(xc * rs * mod_v[4 * D:5 * D, :] + mod_v[3 * D:4 * D, :])
        return xc * rs

    def inv_body(i, carry):
        ha, hb = token_tile(i), token_tile(i + NT // 2)
        for n, op in enumerate(_lhs_operands(ha[0:HD], hb[0:HD], ha[HD:D], hb[HD:D])):
            a1_v[n, :, lanes(i)] = op.astype(bf16)
        return carry

    jax.lax.fori_loop(0, NT // 2, inv_body, 0)

    def bias(ref, t0, n):
        return jnp.concatenate([ref[pl.ds(t0 + t, 1), :] for t in range(n)], axis=1)

    def mm1_body(j, carry):
        cp_w1(j, 0).wait()
        cp_w1(j, 1).wait()

        @pl.when(j == 2)
        def _():
            cp_w2.start()

        c0, c1 = lanes(j, FC), lanes(j + N1, FC)
        quad = {}

        def emit(rh, ch, u):
            quad[rh, ch] = _gelu(u + bias(b1_f, (j + ch * N1) * (FC // L), FC // L))

        _strassen(lambda n: a1_v[n],
                  lambda: w1_v[0:S // 2, c0], lambda: w1_v[0:S // 2, c1],
                  lambda: w1_v[S // 2:S, c0], lambda: w1_v[S // 2:S, c1], emit)
        for n, op in enumerate(_lhs_operands(quad[0, 0], quad[0, 1], quad[1, 0], quad[1, 1])):
            a2_v[n, :, c0] = op.astype(bf16)
        return carry

    jax.lax.fori_loop(0, N1, mm1_body, 0)

    cp_w2.wait()

    def mm2_body(j, carry):
        c0, c1 = lanes(j, SC), lanes(j + N2, SC)

        def emit(rh, ch, y):
            rows, cols = slice(rh * HD, (rh + 1) * HD), (c0, c1)[ch]
            gate = mod_v[5 * D + rh * HD:5 * D + (rh + 1) * HD, :]
            gate = jnp.concatenate([gate] * (SC // L), axis=1)
            y = y + bias(b2_f, (j + ch * N2) * (SC // L), SC // L)
            o_v[rows, cols] = (x1_v[rows, cols] + gate * y).astype(bf16)

        _strassen(lambda n: a2_v[n],
                  lambda: w2_v[0:F // 2, c0], lambda: w2_v[0:F // 2, c1],
                  lambda: w2_v[F // 2:F, c0], lambda: w2_v[F // 2:F, c1], emit)
        cp_o(j, 0).start()
        cp_o(j, 1).start()
        return carry

    jax.lax.fori_loop(0, N2, mm2_body, 0)
    for j in range(N2):
        cp_o(j, 0).wait()
        cp_o(j, 1).wait()


@jax.jit
def pallas_adaLN_cond__spectral_gfnet__mixer_token_mlp__prompt_kernel(
    A_x: jax.Array,
    A_w_r: jax.Array,
    A_w_i: jax.Array,
    B_x: jax.Array,
    B_w1: jax.Array,
    B_b1: jax.Array,
    B_w2: jax.Array,
    B_b2: jax.Array,
    c: jax.Array,
    w_mod: jax.Array,
):
    del B_x
    outT = pl.pallas_call(
        _kernel,
        out_shape=jax.ShapeDtypeStruct((D, S), bf16),
        in_specs=[pl.BlockSpec(memory_space=pl.ANY)] * 10,
        out_specs=pl.BlockSpec(memory_space=pl.ANY),
        scratch_shapes=[
            pltpu.VMEM((D, S), bf16),
            pltpu.VMEM((DF, S), bf16),
            pltpu.VMEM((DF, S), bf16),
            pltpu.VMEM((S, F), bf16),
            pltpu.VMEM((F // L, L), bf16),
            pltpu.VMEM((F, S), bf16),
            pltpu.VMEM((NT, L), bf16),
            pltpu.VMEM((1, D), bf16),
            pltpu.VMEM((D, 6 * D), bf16),
            pltpu.VMEM((10, L, L), bf16),
            pltpu.VMEM((F // L, L), f32),
            pltpu.VMEM((NT, L), f32),
            pltpu.VMEM((6 * D, L), f32),
            pltpu.VMEM((NT, 3, L, L), bf16),
            pltpu.VMEM((NT, 2, 152, L), u32),
            pltpu.VMEM((NT, 2, R, L), f32),
            pltpu.VMEM((NT, 3, R, L), bf16),
            pltpu.VMEM((NT, 2, R, L), bf16),
            pltpu.VMEM((D, S), f32),
            pltpu.VMEM((7, HD, S // 2), bf16),
            pltpu.VMEM((7, HD, F // 2), bf16),
            pltpu.VMEM((D, S), bf16),
            pltpu.SemaphoreType.DMA((9,)),
            pltpu.SemaphoreType.DMA((XC,)),
            pltpu.SemaphoreType.DMA((2 * N1,)),
            pltpu.SemaphoreType.DMA((2 * N2,)),
        ],
        compiler_params=pltpu.CompilerParams(vmem_limit_bytes=112 * 1024 * 1024),
        name="adaln_gfnet_token_mlp",
    )(A_x[0].T, A_w_r.T, A_w_i.T, B_w1, B_b1.reshape(F // L, L), B_w2, B_b2.reshape(NT, L), c, w_mod,
      jnp.asarray(_DMAT, bf16))
    return outT.T[None]
```

```python
import numpy as np

import jax
import jax.numpy as jnp
import jax.experimental.pallas as pl
import jax.experimental.pallas.tpu as pltpu

S, D, F = 2048, 576, 4608
DF = D // 2 + 1
L = 128
NT = S // L
RA, RB = 144, 152
EPS = 1e-5
f32, bf16, u32 = jnp.float32, jnp.bfloat16, jnp.uint32

_ORDER = (1, 10, 8, 17, 2, 11, 7, 16, 3, 12, 6, 15, 4, 13, 5, 14, 0, 9)
_S3 = float(np.sqrt(3.0) / 2)
_C1, _C2, _C4 = (float(np.cos(2 * np.pi * k / 9)) for k in (1, 2, 4))
_S1, _S2, _S4 = (float(np.sin(2 * np.pi * k / 9)) for k in (1, 2, 4))


def _channel_dft_matrices():
    dp = np.arange(64)
    ca, cb = (dp // 8) * 16 + dp % 8, (dp // 8) * 16 + dp % 8 + 8
    fw = np.zeros((5, 128, 128))
    iv = np.zeros((5, 128, 128))
    for h in range(2):
        for m in range(8):
            for g in range(4):
                r = g + 1
                bs = _S3 if r == 3 else 1.0
                for q in range(4):
                    rho = _ORDER[4 * g + q]
                    sig = 1.0 if rho % 9 == r else -1.0
                    phi = 2 * np.pi * dp * (18 * (8 * h + m) + rho) / D
                    re = 32 * h + 8 * q + m
                    im = 64 + re
                    fw[g, re, ca], fw[g, re, cb] = np.cos(phi), -sig * bs * np.sin(phi)
                    fw[g, im, ca], fw[g, im, cb] = -np.sin(phi), -sig * bs * np.cos(phi)
                    c = 2.0 / (D * S)
                    iv[g, ca, re], iv[g, ca, im] = c * np.cos(phi), -c * np.sin(phi)
                    iv[g, cb, re], iv[g, cb, im] = bs * sig * c * np.sin(phi), bs * sig * c * np.cos(phi)
            for q in range(2):
                kd = 18 * (8 * h + m) + _ORDER[16 + q]
                phi = 2 * np.pi * dp * kd / D
                re = 16 * h + 8 * q + m
                im = 40 + re
                c = (1.0 if kd == 0 else 2.0) / (D * S)
                fw[4, re, :64], fw[4, im, :64] = np.cos(phi), -np.sin(phi)
                iv[4, :64, re], iv[4, :64, im] = c * np.cos(phi), -c * np.sin(phi)
    fw[4, 32, :64] = np.cos(np.pi * dp)
    iv[4, :64, 32] = np.cos(np.pi * dp) / (D * S)
    return np.concatenate([fw, iv], 0).astype(np.float32)


_DMAT = _channel_dft_matrices()


def _radix9(h0, p1, p2, p3, p4, m1, m2, q, m4):
    e = p1 + p2 + p4
    f = h0 + p3
    base = h0 - 0.5 * p3
    a, b = p1 - p4, p2 - p4
    r1, r2 = _C1 * a + _C2 * b, _C2 * a + _C4 * b
    u, v = m1 + m2, m2 + m4
    i1, i2 = _S1 * u + _S4 * v, _S2 * u - _S1 * v
    return ((f + e, base + r1, base + r2, f - 0.5 * e, base - (r1 + r2)),
            (i1 + q, i2 - q, m1 - m2 + m4, (i2 - i1) + q))


def _radix4(x0, x1, x2, x3, inverse):
    t0 = (x0[0] + x2[0], x0[1] + x2[1])
    t1 = (x0[0] - x2[0], x0[1] - x2[1])
    return _radix4_tail(t0, t1, x1, x3, inverse)


def _radix4_tail(t0, t1, x1, x3, inverse):
    t2 = (x1[0] + x3[0], x1[1] + x3[1])
    t3 = (x1[0] - x3[0], x1[1] - x3[1])
    ya = (t1[0] + t3[1], t1[1] - t3[0])
    yb = (t1[0] - t3[1], t1[1] + t3[0])
    if inverse:
        ya, yb = yb, ya
    return [(t0[0] + t2[0], t0[1] + t2[1]), ya, (t0[0] - t2[0], t0[1] - t2[1]), yb]


def _twiddle16(z, n, inverse):
    if n == 0:
        return z
    c = float(np.cos(2 * np.pi * n / 16))
    s = float(np.sin(2 * np.pi * n / 16)) * (-1.0 if inverse else 1.0)
    re, im = z
    if n % 4 == 2:
        if c * s > 0:
            return ((re + im) * c, (im - re) * c)
        return ((re - im) * c, (im + re) * c)
    return (re * c + im * s, im * c - re * s)


def _fft16(load, store, inverse):
    a = [_radix4(load(a0), load(4 + a0), load(8 + a0), load(12 + a0), inverse) for a0 in range(4)]
    for k0 in range(4):
        x0, x1, x3 = a[0][k0], _twiddle16(a[1][k0], k0, inverse), _twiddle16(a[3][k0], 3 * k0, inverse)
        if k0 == 2:
            x2 = a[2][k0]
            ta, tb = (x0[0] + x2[1], x0[1] - x2[0]), (x0[0] - x2[1], x0[1] + x2[0])
            t0, t1 = (tb, ta) if inverse else (ta, tb)
            y = _radix4_tail(t0, t1, x1, x3, inverse)
        else:
            y = _radix4(x0, x1, _twiddle16(a[2][k0], 2 * k0, inverse), x3, inverse)
        for k1 in range(4):
            store(k0 + 4 * k1, y[k1])


def _dot(a, b):
    return jnp.dot(a, b, preferred_element_type=f32)


def _dot_nt(a, b):
    return jax.lax.dot_general(a, b, (((1,), (1,)), ((), ())), preferred_element_type=f32)


def _col_mean(acc):
    part = acc[0:8]
    for i in range(8, acc.shape[0], 8):
        part = part + acc[i:i + 8]
    return jnp.broadcast_to(jnp.sum(part, axis=0, keepdims=True) * (1.0 / D), part.shape)


def _rows(x, n):
    return jnp.concatenate([x] * n, axis=0)


def _cols(x, n):
    return jnp.concatenate([x] * n, axis=1)


def _gelu(x):
    k = float(np.sqrt(2 / np.pi))
    t = jnp.tanh(x * (x * x * (k * 0.044715) + k))
    hx = 0.5 * x
    return hx * t + hx


def _pack(x):
    return pltpu.bitcast(x.astype(bf16), u32)


def _unpack(x):
    return pltpu.bitcast(x, bf16)


def _lhs_operands(a11, a12, a21, a22):
    return (a11 + a22, a21 + a22, a11, a22, a11 + a12, a21 - a11, a12 - a22)


def _lhs_operands2(a):
    outer = [_lhs_operands(a[p][q], a[p][q + 2], a[p + 2][q], a[p + 2][q + 2]) for p in range(2) for q in range(2)]
    return [op for four in zip(*outer) for op in _lhs_operands(*four)]


def _strassen(product, b, add, sub, emit):
    m5 = product(4, b(1, 1))
    m3 = product(2, sub(b(0, 1), b(1, 1)))
    emit(0, 1, add(m3, m5))
    m2 = product(1, b(0, 0))
    c22 = sub(m3, m2)
    m4 = product(3, sub(b(1, 0), b(0, 0)))
    emit(1, 0, add(m2, m4))
    c11 = sub(m4, m5)
    m1 = product(0, add(b(0, 0), b(1, 1)))
    c11, c22 = add(c11, m1), add(c22, m1)
    emit(0, 0, add(c11, product(6, add(b(1, 0), b(1, 1)))))
    emit(1, 1, add(c22, product(5, add(b(0, 0), b(0, 1)))))


def _strassen2(lhs, rhs, emit, after=None):
    quads = [(p, q) for p in range(2) for q in range(2)]
    order = iter(range(49))

    def add(x, y):
        return x.astype(f32) + y.astype(f32)

    def sub(x, y):
        return x.astype(f32) - y.astype(f32)

    def inner(i, b):
        out = {}

        def product(k, w):
            m = _dot(lhs(7 * i + k), w.astype(bf16))
            if after is not None:
                after(next(order), m)
            return m

        _strassen(product, lambda p, q: b[p, q], add, sub,
                  lambda p, q, value: out.__setitem__((p, q), value))
        return out

    _strassen(inner, lambda p, q: {pq: rhs(2 * p + pq[0], 2 * q + pq[1]) for pq in quads},
              lambda x, y: {pq: add(x[pq], y[pq]) for pq in quads},
              lambda x, y: {pq: sub(x[pq], y[pq]) for pq in quads},
              lambda p, q, value: [emit(2 * p + pq[0], 2 * q + pq[1], value[pq]) for pq in value])


def _interleave(main, side):
    done = 0
    for i, job in enumerate(main):
        job()
        upto = (i + 1) * len(side) // len(main)
        for s in side[done:upto]:
            s()
        done = upto


XC = 8
RU = 4
XT = NT // XC
QD = D // 4
N1 = F // 4 // L
N2 = S // 4 // L
M_A, M_B, M_C = 2 * D // L, -(-5 * D // L), 6 * D // L


def _kernel(xT_hbm, wr_hbm, wi_hbm, w1_hbm, b1_hbm, w2_hbm, b2_hbm, c_hbm, wm_hbm, dm_hbm, o_hbm,
            x_v, w_v, w1_v, b1_v, w2_v, b2_v, c_v, wm_v, dm_v,
            dm_f, b1_f, b2_f, mod_v, t_v, wpa_v, wpb_v, ha_v, hb_v, ga_v, gb_v, ta_v, tb_v, st_v, h2_v, x1_v, a1_v, a2_v, o_v,
            sem, sem_x, sem_w1, sem_w2, sem_o):
    def lanes(i, n=L):
        return pl.ds(pl.multiple_of(i * n, n), n)

    def copy(src, dst, i):
        return pltpu.make_async_copy(src, dst, sem.at[i])

    def cp_wm(t0, t1, i):
        return copy(wm_hbm.at[:, t0 * L:t1 * L], wm_v.at[:, t0 * L:t1 * L], i)

    cp_c, cp_dm = copy(c_hbm, c_v, 0), copy(dm_hbm, dm_v, 1)
    cp_wma, cp_wmb, cp_wmc = cp_wm(0, M_A, 2), cp_wm(M_A, M_B, 3), cp_wm(M_B, M_C, 4)
    cp_wa = [copy(w.at[0:RA], w_v.at[z, 0:RA], 5 + z) for z, w in enumerate((wr_hbm, wi_hbm))]
    cp_wb = [copy(w.at[RA:DF], w_v.at[z, RA:DF], 7 + z) for z, w in enumerate((wr_hbm, wi_hbm))]
    cp_b1, cp_b2 = copy(b1_hbm, b1_v, 9), copy(b2_hbm, b2_v, 10)

    def cp_x(a):
        return pltpu.make_async_copy(xT_hbm.at[:, lanes(a)], x_v.at[a], sem_x.at[a])

    def cp_w1(j, q):
        return pltpu.make_async_copy(w1_hbm.at[:, lanes(j + q * N1)], w1_v.at[j, q], sem_w1.at[j + q * N1])

    def cp_w2(a):
        return pltpu.make_async_copy(w2_hbm.at[:, lanes(a)], w2_v.at[a], sem_w2.at[a])

    def cp_o(a, h):
        rows = slice(h * D // 2, (h + 1) * D // 2)
        return pltpu.make_async_copy(o_v.at[a, rows], o_hbm.at[rows, lanes(a)], sem_o.at[2 * a + h])

    def loop(n, body):
        jax.lax.fori_loop(0, n, lambda i, c: (body(i), c)[1], 0)

    def start_in_order(copies):
        loop(len(copies), lambda i: [pl.when(i == k)(cp.start) for k, cp in enumerate(copies)])

    start_in_order([cp_c, cp_wma, cp_dm])
    loop(NT, lambda a: cp_x(a).start())
    start_in_order(cp_wa + cp_wb + [cp_wmb, cp_b1, cp_b2])

    row = jax.lax.broadcasted_iota(jnp.int32, (L, L), 0)
    row = ((row & 63) << 1) | (row >> 6)
    lane = jax.lax.broadcasted_iota(jnp.int32, (L, L), 1)
    ang = ((row * (8 * (lane & 15) + (lane >> 4))) & 127).astype(f32) * float(2 * np.pi / L)
    step = row.astype(f32) * float(2 * np.pi / S)
    ec, es = jnp.cos(step), jnp.sin(step)
    tc, ts = jnp.cos(ang), jnp.sin(ang)
    for k1 in range(NT):
        for n, m in enumerate((tc, tc - ts, -ts - tc)):
            m = pltpu.pack_elementwise([m[0:L // 2], m[L // 2:L]], packed_dtype=bf16)
            t_v[k1, n] = pltpu.roll(m, k1, 1) if k1 else m
        tc, ts = tc * ec - ts * es, ts * ec + tc * es

    cp_c.wait()
    cf = c_v[...].astype(f32)
    sc = jnp.broadcast_to(cf * jax.nn.sigmoid(cf), (8, D))

    def modulation(t):
        m = _dot(sc, wm_v[:, t * L:(t + 1) * L])
        col = _rows(m, L // 8).T
        for r0, r1 in ((0, L // 2), (L // 2, L)):
            one = 1.0 if (t * L + r0) // D in (1, 4) else 0.0
            mod_v[t * L + r0:t * L + r1, :] = col[r0:r1] + one if one else col[r0:r1]

    with jax.named_scope("w_wma"):
        cp_wma.wait()
    with jax.named_scope("mod_a"):
        for t in range(M_A):
            modulation(t)
    cp_dm.wait()
    dm_f[...] = dm_v[...].astype(f32)

    def channel_dft(i):
        for t in range(XT):
            a = i * XT + t
            for g in range(4):
                o = _dot(dm_f[g], ta_v[t, 128 * g:128 * g + 128, :])
                for z in range(2):
                    ha_v[a, z, 32 * g:32 * g + 32, :] = o[64 * z:64 * z + 32]
                    hb_v[a, z, 32 * g:32 * g + 32, :] = o[64 * z + 32:64 * z + 64]
            o = _dot(dm_f[4, 0:72, 0:64], ta_v[t, 512:D, :])
            ha_v[a, 0, 128:RA, :] = o[0:16]
            hb_v[a, 0, 128:RB, :] = o[16:40]
            ha_v[a, 1, 128:RA, :] = o[40:56]
            hb_v[a, 1, 128:RA, :] = o[56:72]
            hb_v[a, 1, RA:RB, :] = jnp.zeros((8, L), f32)

    def ln_stats(i):
        for t in range(XT):
            a = i * XT + t
            pivot = jnp.broadcast_to(x_v[a, 0:1, :].astype(f32), (32, L))
            s1 = s2 = None
            for r in range(0, D, 32):
                d = x_v[a, r:r + 32, :].astype(f32) - pivot
                s1, s2 = (d, d * d) if r == 0 else (s1 + d, s2 + d * d)
            m1 = _col_mean(s1)
            st_v[t, 0] = pivot[0:8] + m1
            st_v[t, 1] = jax.lax.rsqrt(jnp.maximum(_col_mean(s2) - m1 * m1, 0.0) + EPS)

    def ln_radix9(i):
        for r in range(0, 64, 8):
            for t in range(XT):
                mean, rstd = st_v[t, 0], st_v[t, 1]
                hb = [(x_v[i * XT + t, q:q + 8, :].astype(f32) - mean) * rstd * mod_v[D + q:D + q + 8, :]
                      + mod_v[q:q + 8, :] for q in range(r, D, 64)]
                p = [hb[j] + hb[9 - j] for j in range(1, 5)]
                m = [hb[j] - hb[9 - j] for j in range(1, 5)]
                ev, od = _radix9(hb[0], p[0], p[1], p[2], p[3], m[0], m[1], _S3 * m[2], m[3])
                for g in range(4):
                    ta_v[t, 128 * g + 2 * r:128 * g + 2 * r + 8, :] = ev[g + 1]
                    ta_v[t, 128 * g + 2 * r + 8:128 * g + 2 * r + 16, :] = od[g]
                ta_v[t, 512 + r:512 + r + 8, :] = ev[0]

    def wait_x(i):
        for t in range(XT):
            cp_x(i * XT + t).wait()

    def fwd_step(i):
        @pl.when(i % 2 == 0)
        def _():
            wait_x(i // 2)
            channel_dft(i // 2 - 1)
            ln_stats(i // 2)

        @pl.when(i % 2 == 1)
        def _():
            ln_radix9(i // 2)

    with jax.named_scope("fwd"):
        wait_x(0)
        ln_stats(0)
        loop(2 * XC - 1, lambda i: fwd_step(i + 1))
        channel_dft(XC - 1)
    loop(N1, lambda j: [cp_w1(j, q).start() for q in range(4)])
    cp_wmc.start()
    loop(NT, lambda a: cp_w2(a).start())

    def radix16(src, dst, p, inverse, tie=None):
        rows = slice(8 * p, 8 * p + 8) if isinstance(p, int) else lanes(p, 8)

        def load(a):
            x = (src[a, 0, rows, :], src[a, 1, rows, :])
            if tie is not None and a < 8:
                q = 32 * (a % 4) + 16 * (a // 4)
                x = (jnp.where(always, x[0], tie[q:q + 8]), jnp.where(always, x[1], tie[q + 8:q + 16]))
            return x

        def store(k, y):
            dst[k, 0, rows, :] = y[0]
            dst[k, 1, rows, :] = y[1]

        _fft16(load, store, inverse)

    def dft128(src, dst, k):
        gr, gi = src[k, 0], src[k, 1]
        p1 = _dot(gr + gi, _unpack(t_v[k, 0]))
        xr = p1 - _dot(gi, _unpack(t_v[k, 1]))
        dst[k, 0] = xr
        dst[k, 1] = p1 + _dot(gr, _unpack(t_v[k, 2]))
        return xr

    lane8 = jax.lax.broadcasted_iota(jnp.int32, (8, L), 1)

    def permute(tiles, dst, z, rows):
        rot = [tiles[0]] + [pltpu.roll(tiles[j], j, 1) for j in range(1, NT)]
        cur = [rot[-i % NT] for i in range(NT)]
        for b in range(4):
            mask = ((lane8 >> b) & 1) == 1
            cur = [jnp.where(mask, cur[(i - (1 << b)) % NT], cur[i]) for i in range(NT)]
        for k in range(NT):
            dst[k, z, rows, :] = cur[k]

    def permute_rows(dst, z, r0, p):
        permute([pltpu.bitcast(w_v[z, r0 + 16 * p:r0 + 16 * p + 16, j * L:(j + 1) * L], u32) for j in range(NT)],
                dst, z, slice(8 * p, 8 * p + 8))

    def permute_nyquist(z):
        nyq = w_v[z, DF - 1:DF, :].astype(f32)
        permute([pltpu.bitcast(jnp.broadcast_to(nyq[:, j * L:(j + 1) * L], (8, L)), u32) for j in range(NT)],
                wpb_v, z, slice(72, 80))

    def idft128(src, wp, dst, k):
        def filt(z):
            blocks = []
            for rho in _ORDER:
                w = wp[k, z, pl.ds(rho // 2, 8, stride=9), :]
                blocks.append(pltpu.bitcast((w & u32(0xFFFF0000)) if rho % 2 else (w << 16), f32))
            if wp is wpb_v:
                blocks.append(pltpu.bitcast(wp[k, z, 72:80, :], f32))
            return jnp.concatenate(blocks, axis=0)

        xr, xi, wr, wi = src[k, 0], src[k, 1], filt(0), filt(1)
        yr, yi = xr * wr - xi * wi, xr * wi + xi * wr
        q1 = _dot_nt(yr + yi, _unpack(t_v[k, 0]))
        zr = q1 + _dot_nt(yi, _unpack(t_v[k, 2]))
        dst[k, 0] = zr
        dst[k, 1] = q1 - _dot_nt(yr, _unpack(t_v[k, 1]))
        return zr

    always = st_v[0, 1] >= 0.0

    def mxu_with_radix16(mxu, src, dst, n, inverse):
        for p in range(n - NT):
            radix16(src, dst, p, inverse)
        for k in range(NT):
            radix16(src, dst, n - NT + k, inverse, mxu(k))

    with jax.named_scope("s1"):
        loop(6, lambda i: [radix16(ha_v, ga_v, 3 * i + t, False) for t in range(3)])
    with jax.named_scope("s2"):
        mxu_with_radix16(lambda k: dft128(ga_v, ha_v, k), hb_v, gb_v, RB // 8, False)
    with jax.named_scope("w_wa"):
        for cp in cp_wa:
            cp.wait()
    with jax.named_scope("s3"):
        loop(2, lambda i: _interleave([lambda t=t: dft128(gb_v, hb_v, 8 * i + t) for t in range(8)],
                                      [lambda t=t: permute_rows(wpa_v, i, 0, t) for t in range(9)]))
    with jax.named_scope("w_wb"):
        for cp in cp_wb:
            cp.wait()
    with jax.named_scope("s4"):
        loop(2, lambda i: _interleave([lambda t=t: idft128(ha_v, wpa_v, ga_v, 8 * i + t) for t in range(8)],
                                      [lambda t=t: permute_rows(wpb_v, i, RA, t) for t in range(9)]
                                      + [lambda: permute_nyquist(i)]))
    with jax.named_scope("s5"):
        mxu_with_radix16(lambda k: idft128(hb_v, wpb_v, gb_v, k), ga_v, ha_v, RA // 8, True)
    with jax.named_scope("w_wmb"):
        cp_wmb.wait()
    with jax.named_scope("s6"):
        _interleave([lambda t=t: radix16(gb_v, hb_v, t, True) for t in range(RB // 8)],
                    [lambda t=t: modulation(t) for t in range(M_A, M_B)])
    cp_b1.wait()
    cp_b2.wait()
    b1_f[...] = b1_v[...].astype(f32)
    b2_f[...] = b2_v[...].astype(f32)

    def inv_pair(i, half):
        tiles = (i + half * NT // 2, i + half * NT // 2 + NT // 4)
        sums = []
        for t, a in enumerate(tiles):
            o = [_dot(dm_f[5 + g], jnp.concatenate(
                [ref[a, z, 32 * g:32 * g + 32, :] for z in range(2) for ref in (ha_v, hb_v)], axis=0))
                for g in range(4)]
            w0 = _dot(dm_f[9, 0:64, 0:72], jnp.concatenate(
                [ha_v[a, 0, 128:RA, :], hb_v[a, 0, 128:RB, :], ha_v[a, 1, 128:RA, :], hb_v[a, 1, 128:RA, :]], axis=0))
            acc = [None] * 3
            for r in range(0, 64, 8):
                al = [o[g][2 * r:2 * r + 8] for g in range(4)]
                be = [o[g][2 * r + 8:2 * r + 16] for g in range(4)]
                ev, od = _radix9(w0[r:r + 8], *al, *be)
                od = (od[0], od[1], _S3 * od[2], od[3])
                y = [ev[0]] + [ev[j + 1] - od[j] for j in range(4)] + [ev[j + 1] + od[j] for j in (3, 2, 1, 0)]
                for j in range(9):
                    q = 64 * j + r
                    x1 = x_v[a, q:q + 8, :].astype(f32) + mod_v[2 * D + q:2 * D + q + 8, :] * y[j]
                    x1_v[a, q:q + 8, :] = x1
                    acc[j % 3] = x1 if acc[j % 3] is None else acc[j % 3] + x1
            sums.append(acc[0] + acc[1] + acc[2])

        def sweep(fn):
            acc = [None, None]
            for r in range(0, D, 32):
                for t in range(2):
                    v = fn(t, slice(r, r + 32))
                    acc[t] = v if r == 0 else acc[t] + v
            return [_rows(_col_mean(v), 4) for v in acc]

        def center(load, mean):
            def fn(t, rows):
                c = load(t, rows) - mean[t]
                ta_v[t, rows, :] = c
                return c * c
            return [jax.lax.rsqrt(v + EPS) for v in sweep(fn)]

        def modulate(t, rows):
            z = (ta_v[t, rows, :] * rstd[t] * mod_v[4 * D + rows.start:4 * D + rows.stop, :]
                 + mod_v[3 * D + rows.start:3 * D + rows.stop, :])
            tb_v[t, rows, :] = z
            return z

        rstd = center(lambda t, rows: x1_v[tiles[t], rows, :], [_rows(_col_mean(v), 4) for v in sums])
        rstd = center(lambda t, rows: tb_v[t, rows, :], sweep(modulate))
        for r in range(0, D, 32):
            for t in range(2):
                h2_v[2 * half + t, r:r + 32, :] = ta_v[t, r:r + 32, :] * rstd[t]

    def left_operands(dst, slot, r, tie=None):
        blocks = [[h2_v[q, QD * p + r:QD * p + r + 16, :] for q in range(4)] for p in range(4)]
        if tie is not None:
            for p, q in ((p, q) for p in range(4) for q in range(4) if p // 2 == q // 2):
                blocks[p][q] = jnp.where(_rows(always, 2), blocks[p][q], tie)
        for n, op in enumerate(_lhs_operands2(blocks)):
            dst[slot, n, r:r + 16, :] = op.astype(bf16)

    def inv_body(i):
        loop(2, lambda half: inv_pair(i, half))
        for r in range(0, QD, 16):
            left_operands(a1_v, i, r)

    with jax.named_scope("inv"):
        loop(NT // 4, inv_body)

    def mm1_body(j):
        for q in range(4):
            cp_w1(j, q).wait()

        def emit(p, q, u):
            h2_v[q, p * QD:(p + 1) * QD, :] = _gelu(u + b1_f[pl.ds(j + q * N1, 1), :])

        def after(n, m):
            if n < QD // 16:
                left_operands(a2_v, (j + N1 - 1) % N1, 16 * n, m[0:16])

        _strassen2(lambda n: jnp.concatenate([a1_v[k, n] for k in range(N2)], axis=1),
                   lambda p, q: w1_v[j, q, p * S // 4:(p + 1) * S // 4, :], emit, after)

    with jax.named_scope("mm1"):
        loop(N1, mm1_body)

    cp_wmc.wait()
    _interleave([lambda r=r: left_operands(a2_v, N1 - 1, r) for r in range(0, QD, 16)],
                [lambda t=t: modulation(t) for t in range(M_B, M_C)])

    def mm2_body(j):
        for q in range(4):
            cp_w2(j + q * N2).wait()
        count = {}

        def emit(p, q, y):
            a, rows = j + q * N2, slice(p * QD, (p + 1) * QD)
            y = y + b2_f[pl.ds(a, 1), :]
            o_v[a, rows, :] = (x1_v[a, rows, :] + mod_v[5 * D + p * QD:5 * D + (p + 1) * QD, :] * y).astype(bf16)
            count[p // 2, q] = count.get((p // 2, q), 0) + 1
            if count[p // 2, q] == 2:
                cp_o(a, p // 2).start()

        _strassen2(lambda n: jnp.concatenate([a2_v[k, n] for k in range(N1)], axis=1),
                   lambda p, q: w2_v[j + q * N2, p * F // 4:(p + 1) * F // 4, :], emit)

    with jax.named_scope("mm2"):
        loop(N2, mm2_body)
    with jax.named_scope("w_out"):
        loop(NT, lambda a: [cp_o(a, h).wait() for h in range(2)])


@jax.jit
def pallas_adaLN_cond__spectral_gfnet__mixer_token_mlp__prompt_kernel(
    A_x: jax.Array,
    A_w_r: jax.Array,
    A_w_i: jax.Array,
    B_x: jax.Array,
    B_w1: jax.Array,
    B_b1: jax.Array,
    B_w2: jax.Array,
    B_b2: jax.Array,
    c: jax.Array,
    w_mod: jax.Array,
):
    del B_x
    outT = pl.pallas_call(
        _kernel,
        out_shape=jax.ShapeDtypeStruct((D, S), bf16),
        in_specs=[pl.BlockSpec(memory_space=pl.ANY)] * 10,
        out_specs=pl.BlockSpec(memory_space=pl.ANY),
        scratch_shapes=[
            pltpu.VMEM((NT, D, L), bf16),
            pltpu.VMEM((2, DF, S), bf16),
            pltpu.VMEM((N1, 4, S, L), bf16),
            pltpu.VMEM((F // L, L), bf16),
            pltpu.VMEM((NT, F, L), bf16),
            pltpu.VMEM((NT, L), bf16),
            pltpu.VMEM((1, D), bf16),
            pltpu.VMEM((D, 6 * D), bf16),
            pltpu.VMEM((10, L, L), bf16),
            pltpu.VMEM((10, L, L), f32),
            pltpu.VMEM((F // L, L), f32),
            pltpu.VMEM((NT, L), f32),
            pltpu.VMEM((6 * D, L), f32),
            pltpu.VMEM((NT, 3, L // 2, L), u32),
            pltpu.VMEM((NT, 2, 72, L), u32),
            pltpu.VMEM((NT, 2, 80, L), u32),
            pltpu.VMEM((NT, 2, RA, L), f32),
            pltpu.VMEM((NT, 2, RB, L), f32),
            pltpu.VMEM((NT, 2, RA, L), f32),
            pltpu.VMEM((NT, 2, RB, L), f32),
            pltpu.VMEM((2, D, L), f32),
            pltpu.VMEM((2, D, L), f32),
            pltpu.VMEM((2, 2, 8, L), f32),
            pltpu.VMEM((4, D, L), f32),
            pltpu.VMEM((NT, D, L), f32),
            pltpu.VMEM((N2, 49, QD, L), bf16),
            pltpu.VMEM((N1, 49, QD, L), bf16),
            pltpu.VMEM((NT, D, L), bf16),
            pltpu.SemaphoreType.DMA((11,)),
            pltpu.SemaphoreType.DMA((NT,)),
            pltpu.SemaphoreType.DMA((4 * N1,)),
            pltpu.SemaphoreType.DMA((NT,)),
            pltpu.SemaphoreType.DMA((2 * NT,)),
        ],
        compiler_params=pltpu.CompilerParams(vmem_limit_bytes=120 * 1024 * 1024),
        name="adaln_gfnet_token_mlp",
    )(A_x[0].T, A_w_r.T, A_w_i.T, B_w1, B_b1.reshape(F // L, L), B_w2, B_b2.reshape(NT, L), c, w_mod,
      jnp.asarray(_DMAT, bf16))
    return outT.T[None]
```

```python
import numpy as np

import jax
import jax.numpy as jnp
import jax.experimental.pallas as pl
import jax.experimental.pallas.tpu as pltpu

S, D, F = 2048, 576, 4608
DF = D // 2 + 1
L = 128
NT = S // L
RA, RB = 144, 152
EPS = 1e-5
f32, bf16, u32 = jnp.float32, jnp.bfloat16, jnp.uint32

_ORDER = (1, 10, 8, 17, 2, 11, 7, 16, 3, 12, 6, 15, 4, 13, 5, 14, 0, 9)
_S3 = float(np.sqrt(3.0) / 2)
_C1, _C2, _C4 = (float(np.cos(2 * np.pi * k / 9)) for k in (1, 2, 4))
_S1, _S2, _S4 = (float(np.sin(2 * np.pi * k / 9)) / _S3 for k in (1, 2, 4))


def _channel_dft_matrices():
    dp = np.arange(64)
    ca, cb = (dp // 8) * 16 + dp % 8, (dp // 8) * 16 + dp % 8 + 8
    fw = np.zeros((5, 128, 128))
    iv = np.zeros((5, 128, 128))
    for h in range(2):
        for m in range(8):
            for g in range(4):
                r = g + 1
                bs = _S3
                for q in range(4):
                    rho = _ORDER[4 * g + q]
                    sig = 1.0 if rho % 9 == r else -1.0
                    phi = 2 * np.pi * dp * (18 * (8 * h + m) + rho) / D
                    re = 32 * h + 8 * q + m
                    im = 64 + re
                    fw[g, re, ca], fw[g, re, cb] = np.cos(phi), -sig * bs * np.sin(phi)
                    fw[g, im, ca], fw[g, im, cb] = -np.sin(phi), -sig * bs * np.cos(phi)
                    c = 2.0 / (D * S)
                    iv[g, ca, re], iv[g, ca, im] = c * np.cos(phi), -c * np.sin(phi)
                    iv[g, cb, re], iv[g, cb, im] = bs * sig * c * np.sin(phi), bs * sig * c * np.cos(phi)
            for q in range(2):
                kd = 18 * (8 * h + m) + _ORDER[16 + q]
                phi = 2 * np.pi * dp * kd / D
                re = 16 * h + 8 * q + m
                im = 40 + re
                c = (1.0 if kd == 0 else 2.0) / (D * S)
                fw[4, re, :64], fw[4, im, :64] = np.cos(phi), -np.sin(phi)
                iv[4, :64, re], iv[4, :64, im] = c * np.cos(phi), -c * np.sin(phi)
    fw[4, 32, :64] = np.cos(np.pi * dp)
    iv[4, :64, 32] = np.cos(np.pi * dp) / (D * S)
    return np.concatenate([fw, iv], 0).astype(np.float32)


_DMAT = _channel_dft_matrices()


def _radix9(h0, p1, p2, p3, p4, m1, m2, m3, m4):
    e = p1 + p2 + p4
    f = h0 + p3
    base = h0 - 0.5 * p3
    a, b = p1 - p4, p2 - p4
    r1, r2 = _C1 * a + _C2 * b, _C2 * a + _C4 * b
    u, v = m1 + m2, m2 + m4
    i1, i2 = _S1 * u + _S4 * v, _S2 * u - _S1 * v
    return ((f + e, base + r1, base + r2, f - 0.5 * e, base - (r1 + r2)),
            (i1 + m3, i2 - m3, m1 - m2 + m4, (i2 - i1) + m3))


def _radix4(x0, x1, x2, x3, inverse):
    t0 = (x0[0] + x2[0], x0[1] + x2[1])
    t1 = (x0[0] - x2[0], x0[1] - x2[1])
    return _radix4_tail(t0, t1, x1, x3, inverse)


def _radix4_tail(t0, t1, x1, x3, inverse):
    t2 = (x1[0] + x3[0], x1[1] + x3[1])
    t3 = (x1[0] - x3[0], x1[1] - x3[1])
    ya = (t1[0] + t3[1], t1[1] - t3[0])
    yb = (t1[0] - t3[1], t1[1] + t3[0])
    if inverse:
        ya, yb = yb, ya
    return [(t0[0] + t2[0], t0[1] + t2[1]), ya, (t0[0] - t2[0], t0[1] - t2[1]), yb]


def _twiddle16(z, n, inverse):
    if n == 0:
        return z
    c = float(np.cos(2 * np.pi * n / 16))
    s = float(np.sin(2 * np.pi * n / 16)) * (-1.0 if inverse else 1.0)
    re, im = z
    if n % 4 == 2:
        if c * s > 0:
            return ((re + im) * c, (im - re) * c)
        return ((re - im) * c, (im + re) * c)
    return (re * c + im * s, im * c - re * s)


def _fft16(load, store, inverse):
    a = [_radix4(load(a0), load(4 + a0), load(8 + a0), load(12 + a0), inverse) for a0 in range(4)]
    for k0 in range(4):
        x0, x1, x3 = a[0][k0], _twiddle16(a[1][k0], k0, inverse), _twiddle16(a[3][k0], 3 * k0, inverse)
        if k0 == 2:
            x2 = a[2][k0]
            ta, tb = (x0[0] + x2[1], x0[1] - x2[0]), (x0[0] - x2[1], x0[1] + x2[0])
            t0, t1 = (tb, ta) if inverse else (ta, tb)
            y = _radix4_tail(t0, t1, x1, x3, inverse)
        else:
            y = _radix4(x0, x1, _twiddle16(a[2][k0], 2 * k0, inverse), x3, inverse)
        for k1 in range(4):
            store(k0 + 4 * k1, y[k1])


def _dot(a, b):
    return jnp.dot(a, b, preferred_element_type=f32)


def _dot_nt(a, b):
    return jax.lax.dot_general(a, b, (((1,), (1,)), ((), ())), preferred_element_type=f32)


def _col_mean(acc):
    part = acc[0:8]
    for i in range(8, acc.shape[0], 8):
        part = part + acc[i:i + 8]
    return jnp.broadcast_to(jnp.sum(part, axis=0, keepdims=True) * (1.0 / D), part.shape)


def _rows(x, n):
    return jnp.concatenate([x] * n, axis=0)


def _cols(x, n):
    return jnp.concatenate([x] * n, axis=1)


def _gelu(x):
    k = float(np.sqrt(2 / np.pi))
    t = jnp.tanh(x * (x * x * (k * 0.044715) + k))
    hx = 0.5 * x
    return hx * t + hx


def _pack(x):
    return pltpu.bitcast(x.astype(bf16), u32)


def _unpack(x):
    return pltpu.bitcast(x, bf16)


def _lhs_operands(a11, a12, a21, a22):
    return (a11 + a22, a21 + a22, a11, a22, a11 + a12, a21 - a11, a12 - a22)


def _lhs_operands2(a):
    outer = [_lhs_operands(a[p][q], a[p][q + 2], a[p + 2][q], a[p + 2][q + 2]) for p in range(2) for q in range(2)]
    return [op for four in zip(*outer) for op in _lhs_operands(*four)]


def _strassen(product, b, add, sub, emit):
    m5 = product(4, b(1, 1))
    m2 = product(1, b(0, 0))
    m3 = product(2, sub(b(0, 1), b(1, 1)))
    emit(0, 1, add(m3, m5))
    c22 = sub(m3, m2)
    m4 = product(3, sub(b(1, 0), b(0, 0)))
    emit(1, 0, add(m2, m4))
    c11 = sub(m4, m5)
    m1 = product(0, add(b(0, 0), b(1, 1)))
    c11, c22 = add(c11, m1), add(c22, m1)
    emit(0, 0, add(c11, product(6, add(b(1, 0), b(1, 1)))))
    emit(1, 1, add(c22, product(5, add(b(0, 0), b(0, 1)))))


def _strassen2(lhs, rhs, emit, after=None):
    quads = [(p, q) for p in range(2) for q in range(2)]
    order = iter(range(49))

    def add(x, y):
        return x.astype(f32) + y.astype(f32)

    def sub(x, y):
        return x.astype(f32) - y.astype(f32)

    def inner(i, b):
        out = {}

        def product(k, w):
            m = _dot(lhs(7 * i + k), w.astype(bf16))
            if after is not None:
                after(next(order), m)
            return m

        _strassen(product, lambda p, q: b[p, q], add, sub,
                  lambda p, q, value: out.__setitem__((p, q), value))
        return out

    _strassen(inner, lambda p, q: {pq: rhs(2 * p + pq[0], 2 * q + pq[1]) for pq in quads},
              lambda x, y: {pq: add(x[pq], y[pq]) for pq in quads},
              lambda x, y: {pq: sub(x[pq], y[pq]) for pq in quads},
              lambda p, q, value: [emit(2 * p + pq[0], 2 * q + pq[1], value[pq]) for pq in value])


def _interleave(main, side):
    done = 0
    for i, job in enumerate(main):
        job()
        upto = (i + 1) * len(side) // len(main)
        for s in side[done:upto]:
            s()
        done = upto


XC = 8
RU = 4
XT = NT // XC
QD = D // 4
N1 = F // 4 // L
N2 = S // 4 // L
M_A, M_B, M_C = 2 * D // L, -(-5 * D // L), 6 * D // L


def _kernel(xT_hbm, wr_hbm, wi_hbm, w1_hbm, b1_hbm, w2_hbm, b2_hbm, c_hbm, wm_hbm, dm_hbm, o_hbm,
            x_v, w_v, w1_v, w2_v, wm_v, dm_v, dm_f, mod_v, t_v, wpa_v, wpb_v, ha_v,
            hb_v, ga_v, gb_v, ta_v, tb_v, h2_v, x1_v, a1_v, a2_v, o_v, b1_v, b2_v, c_v, b1_f, b2_f, mr_v, st_v,
            sem, sem_x, sem_w1, sem_w2):
    def lanes(i, n=L):
        return pl.ds(pl.multiple_of(i * n, n), n)

    def copy(src, dst, i):
        return pltpu.make_async_copy(src, dst, sem.at[i])

    def cp_wm(t0, t1, i):
        return copy(wm_hbm.at[:, t0 * L:t1 * L], wm_v.at[:, t0 * L:t1 * L], i)

    cp_c, cp_dm = copy(c_hbm, c_v, 0), copy(dm_hbm, dm_v, 1)
    cp_wma, cp_wmb = cp_wm(0, M_A, 2), cp_wm(M_A, M_C, 3)
    cp_wa = [copy(w.at[0:RA], w_v.at[z, 0:RA], 5 + z) for z, w in enumerate((wr_hbm, wi_hbm))]
    cp_wb = [copy(w.at[RA:DF], w_v.at[z, RA:DF], 7 + z) for z, w in enumerate((wr_hbm, wi_hbm))]
    cp_b1, cp_b2 = copy(b1_hbm, b1_v, 9), copy(b2_hbm, b2_v, 10)

    def cp_x(a):
        return pltpu.make_async_copy(xT_hbm.at[:, lanes(a)], x_v.at[a], sem_x.at[a // XT])

    def cp_w1(j, q):
        return pltpu.make_async_copy(w1_hbm.at[:, lanes(j + q * N1)], w1_v.at[j, q], sem_w1.at[j])

    def cp_w2(a):
        return pltpu.make_async_copy(w2_hbm.at[:, lanes(a)], w2_v.at[a], sem_w2.at[a % N2])

    def cp_o(a, h):
        rows = slice(h * D // 2, (h + 1) * D // 2)
        return pltpu.make_async_copy(o_v.at[a, rows], o_hbm.at[rows, lanes(a)], sem.at[4])

    def loop(n, body):
        jax.lax.fori_loop(0, n, lambda i, c: (body(i), c)[1], 0)

    def start_in_order(copies):
        def body(i, total):
            for k, cp in enumerate(copies):
                pl.when(i == k)(cp.start)
            return total + i

        return jax.lax.fori_loop(0, len(copies), body, 0) > 0

    start_in_order([cp_c, cp_wma, cp_dm])
    loop(NT, lambda a: cp_x(a).start())
    yes = start_in_order(cp_wa + cp_wb + [cp_wmb, cp_b1, cp_b2])

    row = jax.lax.broadcasted_iota(jnp.int32, (L, L), 0)
    row = ((row & 63) << 1) | (row >> 6)
    lane = jax.lax.broadcasted_iota(jnp.int32, (L, L), 1)
    ang = ((row * (8 * (lane & 15) + (lane >> 4))) & 127).astype(f32) * float(2 * np.pi / L)
    step = row.astype(f32) * float(2 * np.pi / S)
    ec, es = jnp.cos(step), jnp.sin(step)
    tc, ts = jnp.cos(ang), jnp.sin(ang)
    for k1 in range(NT):
        for n, m in enumerate((tc, tc - ts, -ts - tc)):
            m = pltpu.pack_elementwise([m[0:L // 2], m[L // 2:L]], packed_dtype=bf16)
            t_v[k1, n] = pltpu.roll(m, k1, 1) if k1 else m
        tc, ts = tc * ec - ts * es, ts * ec + tc * es

    cp_c.wait()
    cf = c_v[...].astype(f32)
    sc = jnp.broadcast_to(cf * jax.nn.sigmoid(cf), (8, D))

    def mod_row(t):
        m = _dot(sc, wm_v[:, t * L:(t + 1) * L])
        mr_v[t] = m
        return m

    def mod_col(t):
        col = _rows(mr_v[t], L // 8).T
        for r0, r1 in ((0, L // 2), (L // 2, L)):
            one = (t * L + r0) // D in (1, 4)
            mod_v[t * L + r0:t * L + r1, :] = col[r0:r1] + 1.0 if one else col[r0:r1]

    with jax.named_scope("w_wma"):
        cp_wma.wait()
    with jax.named_scope("mod_a"):
        for t in range(M_A):
            mod_row(t)
            mod_col(t)
    cp_dm.wait()
    dm_f[...] = dm_v[...].astype(f32)

    def channel_dft(i):
        for t in range(XT):
            a = i * XT + t
            for g in range(4):
                o = _dot(dm_f[g], ta_v[t, 128 * g:128 * g + 128, :])
                for z in range(2):
                    ha_v[a, z, 32 * g:32 * g + 32, :] = o[64 * z:64 * z + 32]
                    hb_v[a, z, 32 * g:32 * g + 32, :] = o[64 * z + 32:64 * z + 64]
            o = _dot(dm_f[4, 0:72, 0:64], ta_v[t, 512:D, :])
            ha_v[a, 0, 128:RA, :] = o[0:16]
            hb_v[a, 0, 128:RB, :] = o[16:40]
            ha_v[a, 1, 128:RA, :] = o[40:56]
            hb_v[a, 1, 128:RA, :] = o[56:72]
            hb_v[a, 1, RA:RB, :] = jnp.zeros((8, L), f32)

    def ln_stats(i):
        for t in range(XT):
            a = i * XT + t
            pivot = jnp.broadcast_to(x_v[a, 0:1, :].astype(f32), (32, L))
            s1 = s2 = None
            for r in range(0, D, 32):
                d = x_v[a, r:r + 32, :].astype(f32) - pivot
                s1, s2 = (d, d * d) if r == 0 else (s1 + d, s2 + d * d)
            m1 = _col_mean(s1)
            st_v[t, 0] = pivot[0:8] + m1
            st_v[t, 1] = jax.lax.rsqrt(jnp.maximum(_col_mean(s2) - m1 * m1, 0.0) + EPS)

    def ln_radix9(i):
        for r in range(0, 64, 8):
            for t in range(XT):
                mean, rstd = st_v[t, 0], st_v[t, 1]
                hb = [(x_v[i * XT + t, q:q + 8, :].astype(f32) - mean) * rstd * mod_v[D + q:D + q + 8, :]
                      + mod_v[q:q + 8, :] for q in range(r, D, 64)]
                p = [hb[j] + hb[9 - j] for j in range(1, 5)]
                m = [hb[j] - hb[9 - j] for j in range(1, 5)]
                ev, od = _radix9(hb[0], p[0], p[1], p[2], p[3], m[0], m[1], m[2], m[3])
                for g in range(4):
                    ta_v[t, 128 * g + 2 * r:128 * g + 2 * r + 8, :] = ev[g + 1]
                    ta_v[t, 128 * g + 2 * r + 8:128 * g + 2 * r + 16, :] = od[g]
                ta_v[t, 512 + r:512 + r + 8, :] = ev[0]

    def wait_x(i):
        for t in range(XT):
            cp_x(i * XT + t).wait()

    def fwd_step(i):
        wait_x(i)
        channel_dft(i - 1)
        ln_stats(i)
        ln_radix9(i)
        for q in range(4):
            cp_w1(i, q).start()

    with jax.named_scope("fwd"):
        wait_x(0)
        ln_stats(0)
        ln_radix9(0)
        for q in range(4):
            cp_w1(0, q).start()
        loop(XC - 1, lambda i: fwd_step(i + 1))
        channel_dft(XC - 1)
        for q in range(4):
            cp_w1(XC, q).start()

    def radix16(src, dst, p, inverse, tie=None):
        rows = slice(8 * p, 8 * p + 8) if isinstance(p, int) else lanes(p, 8)

        def load(a):
            x = (src[a, 0, rows, :], src[a, 1, rows, :])
            if tie is not None and a < 8:
                q = 32 * (a % 4) + 16 * (a // 4)
                x = (jnp.where(always, x[0], tie[q:q + 8]), jnp.where(always, x[1], tie[q + 8:q + 16]))
            return x

        def store(k, y):
            dst[k, 0, rows, :] = y[0]
            dst[k, 1, rows, :] = y[1]

        _fft16(load, store, inverse)

    def dft128(src, dst, k):
        gr, gi = src[k, 0], src[k, 1]
        p1 = _dot(gr + gi, _unpack(t_v[k, 0]))
        xr = p1 - _dot(gi, _unpack(t_v[k, 1]))
        dst[k, 0] = xr
        dst[k, 1] = p1 + _dot(gr, _unpack(t_v[k, 2]))
        return xr

    lane8 = jax.lax.broadcasted_iota(jnp.int32, (8, L), 1)

    def permute(tiles, dst, z, rows):
        rot = [tiles[0]] + [pltpu.roll(tiles[j], j, 1) for j in range(1, NT)]
        cur = [rot[-i % NT] for i in range(NT)]
        for b in range(4):
            mask = ((lane8 >> b) & 1) == 1
            cur = [jnp.where(mask, cur[(i - (1 << b)) % NT], cur[i]) for i in range(NT)]
        for k in range(NT):
            dst[k, z, rows, :] = cur[k]

    def permute_rows(dst, z, r0, p):
        permute([pltpu.bitcast(w_v[z, r0 + 16 * p:r0 + 16 * p + 16, j * L:(j + 1) * L], u32) for j in range(NT)],
                dst, z, slice(8 * p, 8 * p + 8))

    def permute_nyquist(z):
        nyq = w_v[z, DF - 1:DF, :].astype(f32)
        permute([pltpu.bitcast(jnp.broadcast_to(nyq[:, j * L:(j + 1) * L], (8, L)), u32) for j in range(NT)],
                wpb_v, z, slice(72, 80))

    def idft128(src, wp, dst, k):
        def filt(z):
            blocks = []
            for rho in _ORDER:
                w = wp[k, z, pl.ds(rho // 2, 8, stride=9), :]
                blocks.append(pltpu.bitcast((w & u32(0xFFFF0000)) if rho % 2 else (w << 16), f32))
            if wp is wpb_v:
                blocks.append(pltpu.bitcast(wp[k, z, 72:80, :], f32))
            return jnp.concatenate(blocks, axis=0)

        xr, xi, wr, wi = src[k, 0], src[k, 1], filt(0), filt(1)
        yr, yi = xr * wr - xi * wi, xr * wi + xi * wr
        q1 = _dot_nt(yr + yi, _unpack(t_v[k, 0]))
        zr = q1 + _dot_nt(yi, _unpack(t_v[k, 2]))
        dst[k, 0] = zr
        dst[k, 1] = q1 - _dot_nt(yr, _unpack(t_v[k, 1]))
        return zr

    always = st_v[0, 1] >= 0.0

    def paced_radix16(jobs, src, dst, n, inverse):
        for p in range(n - len(jobs)):
            radix16(src, dst, p, inverse)
        for p, job in enumerate(jobs):
            radix16(src, dst, n - len(jobs) + p, inverse, job())

    with jax.named_scope("s1"):
        loop(6, lambda i: [radix16(ha_v, ga_v, 3 * i + t, False) for t in range(3)])
    with jax.named_scope("s2"):
        pl.when(yes)(lambda: paced_radix16([lambda k=k: dft128(ga_v, ha_v, k) for k in range(NT)],
                                           hb_v, gb_v, RB // 8, False))
    with jax.named_scope("w_wa"):
        for cp in cp_wa:
            cp.wait()
    with jax.named_scope("s3"):
        pl.when(yes)(lambda: _interleave(
            [lambda k=k: dft128(gb_v, hb_v, k) for k in range(NT)],
            [lambda z=z, p=p: permute_rows(wpa_v, z, 0, p) for z in range(2) for p in range(9)]))
    with jax.named_scope("w_wb"):
        for cp in cp_wb:
            cp.wait()
    with jax.named_scope("s4"):
        pl.when(yes)(lambda: _interleave(
            [lambda k=k: idft128(ha_v, wpa_v, ga_v, k) for k in range(NT)],
            [lambda z=z, p=p: permute_rows(wpb_v, z, RA, p) for z in range(2) for p in range(9)]
            + [lambda z=z: permute_nyquist(z) for z in range(2)]))
    with jax.named_scope("s5"):
        pl.when(yes)(lambda: paced_radix16([lambda k=k: idft128(hb_v, wpb_v, gb_v, k) for k in range(NT)],
                                           ga_v, ha_v, RA // 8, True))
    with jax.named_scope("w_wmb"):
        cp_wmb.wait()
    with jax.named_scope("s6"):
        pl.when(yes)(lambda: paced_radix16([lambda t=t: _rows(mod_row(t), 16) for t in range(M_A, M_C)],
                                           gb_v, hb_v, RB // 8, True))
    cp_b1.wait()
    cp_b2.wait()
    b1_f[...] = b1_v[...].astype(f32)
    b2_f[...] = b2_v[...].astype(f32)

    def pair_tiles(n):
        first = n // 2 + (n % 2) * (NT // 2)
        return first, first + NT // 4

    def channel_idft(n):
        for t, a in enumerate(pair_tiles(n)):
            tb_v[t, 512:D, :] = _dot(dm_f[9, 0:64, 0:72], jnp.concatenate(
                [ha_v[a, 0, 128:RA, :], hb_v[a, 0, 128:RB, :], ha_v[a, 1, 128:RA, :], hb_v[a, 1, 128:RA, :]], axis=0))
            for g in range(4):
                tb_v[t, 128 * g:128 * g + 128, :] = _dot(dm_f[5 + g], jnp.concatenate(
                    [ref[a, z, 32 * g:32 * g + 32, :] for z in range(2) for ref in (ha_v, hb_v)], axis=0))

    def inv_pair(n):
        tiles, sums = pair_tiles(n), []
        for t, a in enumerate(tiles):
            acc = [None] * 3
            for r in range(0, 64, 8):
                al = [tb_v[t, 128 * g + 2 * r:128 * g + 2 * r + 8, :] for g in range(4)]
                be = [tb_v[t, 128 * g + 2 * r + 8:128 * g + 2 * r + 16, :] for g in range(4)]
                ev, od = _radix9(tb_v[t, 512 + r:512 + r + 8, :], *al, *be)
                y = [ev[0]] + [ev[j + 1] - od[j] for j in range(4)] + [ev[j + 1] + od[j] for j in (3, 2, 1, 0)]
                for j in range(9):
                    q = 64 * j + r
                    x1 = x_v[a, q:q + 8, :].astype(f32) + mod_v[2 * D + q:2 * D + q + 8, :] * y[j]
                    x1_v[a, q:q + 8, :] = x1
                    acc[j % 3] = x1 if acc[j % 3] is None else acc[j % 3] + x1
            sums.append(acc[0] + acc[1] + acc[2])
        channel_idft(jnp.minimum(n + 1, NT // 2 - 1))

        def sweep(fn):
            acc = [None, None]
            for r in range(0, D, 32):
                for t in range(2):
                    v = fn(t, slice(r, r + 32))
                    acc[t] = v if r == 0 else acc[t] + v
            return [_rows(_col_mean(v), 4) for v in acc]

        def modulate(t, rows):
            z = ((x1_v[tiles[t], rows, :] - mean[t]) * rstd[t] * mod_v[4 * D + rows.start:4 * D + rows.stop, :]
                 + mod_v[3 * D + rows.start:3 * D + rows.stop, :])
            ta_v[t, rows, :] = z
            return z

        def center(t, rows):
            c = ta_v[t, rows, :] - mean2[t]
            h2_v[2 * (n % 2) + t, rows, :] = c
            return c * c

        mean = [_rows(_col_mean(v), 4) for v in sums]
        rstd = [jax.lax.rsqrt(v + EPS) for v in sweep(lambda t, rows: jnp.square(x1_v[tiles[t], rows, :] - mean[t]))]
        mean2 = sweep(modulate)
        for t, v in enumerate(sweep(center)):
            st_v[n % 2, t] = jax.lax.rsqrt(v[0:8] + EPS)

    def left_operands(dst, slot, r, prep):
        blocks = [[prep(p, q, h2_v[q, pl.ds(QD * p + r, 16), :]) for q in range(4)] for p in range(4)]
        for n, op in enumerate(_lhs_operands2(blocks)):
            dst[slot, n, pl.ds(r, 16), :] = op.astype(bf16)

    def paced(tie):
        return lambda p, q, g: jnp.where(_rows(always, 2), g, tie) if p // 2 == q // 2 else g

    def inv_body(i):
        for q in range(4):
            cp_w2(i + q * N2).start()
        loop(2, lambda half: inv_pair(2 * i + half))
        for r in range(0, QD, 16):
            left_operands(a1_v, i, r, lambda p, q, c: c * _rows(st_v[q // 2, q % 2], 2))

    with jax.named_scope("inv"):
        channel_idft(0)
        for t in range(M_A, M_C):
            mod_col(t)
        loop(NT // 4, inv_body)

    def mm1_body(j):
        with jax.named_scope("w_w1"):
            for q in range(4):
                cp_w1(j, q).wait()

        def emit(p, q, u):
            h2_v[q, p * QD:(p + 1) * QD, :] = _gelu(u + b1_f[pl.ds(j + q * N1, 1), :])

        def after(n, m):
            for r in range(QD // 16):
                if r * 13 // 9 == n:
                    at = 16 * (r * 13 % 9)
                    left_operands(a2_v, (j + N1 - 1) % N1, 16 * r, paced(m[at:at + 16]))

        _strassen2(lambda n: jnp.concatenate([a1_v[k, n] for k in range(N2)], axis=1),
                   lambda p, q: w1_v[j, q, p * S // 4:(p + 1) * S // 4, :], emit, after)

    with jax.named_scope("mm1"):
        loop(N1, mm1_body)

    for r in range(0, QD, 16):
        left_operands(a2_v, N1 - 1, r, lambda p, q, g: g)

    def mm2_body(j):
        for q in range(4):
            cp_w2(j + q * N2).wait()
        done = set()

        def emit(p, q, y):
            a, rows = j + q * N2, slice(p * QD, (p + 1) * QD)
            gate = mod_v[5 * D + rows.start:5 * D + rows.stop, :]
            o_v[a, rows, :] = (x1_v[a, rows, :] + gate * (y + b2_f[pl.ds(a, 1), :])).astype(bf16)
            done.add((p, q))
            if (p ^ 1, q) in done:
                cp_o(a, p // 2).start()

        _strassen2(lambda n: jnp.concatenate([a2_v[k, n] for k in range(N1)], axis=1),
                   lambda p, q: w2_v[j + q * N2, p * F // 4:(p + 1) * F // 4, :], emit)

    with jax.named_scope("mm2"):
        loop(N2, mm2_body)
    with jax.named_scope("w_out"):
        loop(NT, lambda a: [cp_o(a, h).wait() for h in range(2)])


@jax.jit
def pallas_adaLN_cond__spectral_gfnet__mixer_token_mlp__prompt_kernel(
    A_x: jax.Array,
    A_w_r: jax.Array,
    A_w_i: jax.Array,
    B_x: jax.Array,
    B_w1: jax.Array,
    B_b1: jax.Array,
    B_w2: jax.Array,
    B_b2: jax.Array,
    c: jax.Array,
    w_mod: jax.Array,
):
    del B_x
    outT = pl.pallas_call(
        _kernel,
        out_shape=jax.ShapeDtypeStruct((D, S), bf16),
        in_specs=[pl.BlockSpec(memory_space=pl.ANY)] * 10,
        out_specs=pl.BlockSpec(memory_space=pl.ANY),
        scratch_shapes=[
            pltpu.VMEM((NT, D, L), bf16),
            pltpu.VMEM((2, DF, S), bf16),
            pltpu.VMEM((N1, 4, S, L), bf16),
            pltpu.VMEM((NT, F, L), bf16),
            pltpu.VMEM((D, 6 * D), bf16),
            pltpu.VMEM((10, L, L), bf16),
            pltpu.VMEM((10, L, L), f32),
            pltpu.VMEM((6 * D, L), f32),
            pltpu.VMEM((NT, 3, L // 2, L), u32),
            pltpu.VMEM((NT, 2, 72, L), u32),
            pltpu.VMEM((NT, 2, 80, L), u32),
            pltpu.VMEM((NT, 2, RA, L), f32),
            pltpu.VMEM((NT, 2, RB, L), f32),
            pltpu.VMEM((NT, 2, RA, L), f32),
            pltpu.VMEM((NT, 2, RB, L), f32),
            pltpu.VMEM((2, D, L), f32),
            pltpu.VMEM((2, D, L), f32),
            pltpu.VMEM((4, D, L), f32),
            pltpu.VMEM((NT, D, L), f32),
            pltpu.VMEM((N2, 49, QD, L), bf16),
            pltpu.VMEM((N1, 49, QD, L), bf16),
            pltpu.VMEM((NT, D, L), bf16),
            pltpu.VMEM((F // L, L), bf16),
            pltpu.VMEM((NT, L), bf16),
            pltpu.VMEM((1, D), bf16),
            pltpu.VMEM((F // L, L), f32),
            pltpu.VMEM((NT, L), f32),
            pltpu.VMEM((M_C, 8, L), f32),
            pltpu.VMEM((2, 2, 8, L), f32),
            pltpu.SemaphoreType.DMA((11,)),
            pltpu.SemaphoreType.DMA((XC,)),
            pltpu.SemaphoreType.DMA((N1,)),
            pltpu.SemaphoreType.DMA((N2,)),
        ],
        compiler_params=pltpu.CompilerParams(vmem_limit_bytes=120 * 1024 * 1024),
        name="adaln_gfnet_token_mlp",
    )(A_x[0].T, A_w_r.T, A_w_i.T, B_w1, B_b1.reshape(F // L, L), B_w2, B_b2.reshape(NT, L), c, w_mod,
      jnp.asarray(_DMAT, bf16))
    return outT.T[None]
```

```python
import numpy as np

import jax
import jax.numpy as jnp
import jax.experimental.pallas as pl
import jax.experimental.pallas.tpu as pltpu

S, D, F = 2048, 576, 4608
DF = D // 2 + 1
L = 128
NT = S // L
RA, RB = 144, 152
EPS = 1e-5
f32, bf16, u32 = jnp.float32, jnp.bfloat16, jnp.uint32

_ORDER = (1, 10, 8, 17, 2, 11, 7, 16, 3, 12, 6, 15, 4, 13, 5, 14, 0, 9)
_S3 = float(np.sqrt(3.0) / 2)
_C1, _C2, _C4 = (float(np.cos(2 * np.pi * k / 9)) for k in (1, 2, 4))
_S1, _S2, _S4 = (float(np.sin(2 * np.pi * k / 9)) / _S3 for k in (1, 2, 4))


def _channel_dft_matrices():
    dp = np.arange(64)
    ca, cb = (dp // 8) * 16 + dp % 8, (dp // 8) * 16 + dp % 8 + 8
    fw = np.zeros((5, 128, 128))
    iv = np.zeros((5, 128, 128))
    for h in range(2):
        for m in range(8):
            for g in range(4):
                r = g + 1
                bs = _S3
                for q in range(4):
                    rho = _ORDER[4 * g + q]
                    sig = 1.0 if rho % 9 == r else -1.0
                    phi = 2 * np.pi * dp * (18 * (8 * h + m) + rho) / D
                    re = 32 * h + 8 * q + m
                    im = 64 + re
                    fw[g, re, ca], fw[g, re, cb] = np.cos(phi), -sig * bs * np.sin(phi)
                    fw[g, im, ca], fw[g, im, cb] = -np.sin(phi), -sig * bs * np.cos(phi)
                    c = 2.0 / (D * S)
                    iv[g, ca, re], iv[g, ca, im] = c * np.cos(phi), -c * np.sin(phi)
                    iv[g, cb, re], iv[g, cb, im] = bs * sig * c * np.sin(phi), bs * sig * c * np.cos(phi)
            for q in range(2):
                kd = 18 * (8 * h + m) + _ORDER[16 + q]
                phi = 2 * np.pi * dp * kd / D
                re = 16 * h + 8 * q + m
                im = 40 + re
                c = (1.0 if kd == 0 else 2.0) / (D * S)
                fw[4, re, :64], fw[4, im, :64] = np.cos(phi), -np.sin(phi)
                iv[4, :64, re], iv[4, :64, im] = c * np.cos(phi), -c * np.sin(phi)
    fw[4, 32, :64] = np.cos(np.pi * dp)
    iv[4, :64, 32] = np.cos(np.pi * dp) / (D * S)
    return np.concatenate([fw, iv], 0).astype(np.float32).astype(bf16)


_DMAT = _channel_dft_matrices()


def _radix9(h0, p1, p2, p3, p4, m1, m2, m3, m4):
    e = p1 + p2 + p4
    f = h0 + p3
    base = h0 - 0.5 * p3
    a, b = p1 - p4, p2 - p4
    r1, r2 = _C1 * a + _C2 * b, _C2 * a + _C4 * b
    u, v = m1 + m2, m2 + m4
    i1, i2 = _S1 * u + _S4 * v, _S2 * u - _S1 * v
    return ((f + e, base + r1, base + r2, f - 0.5 * e, base - (r1 + r2)),
            (i1 + m3, i2 - m3, m1 - m2 + m4, (i2 - i1) + m3))


def _radix4(x0, x1, x2, x3, inverse):
    t0 = (x0[0] + x2[0], x0[1] + x2[1])
    t1 = (x0[0] - x2[0], x0[1] - x2[1])
    return _radix4_tail(t0, t1, x1, x3, inverse)


def _radix4_tail(t0, t1, x1, x3, inverse):
    t2 = (x1[0] + x3[0], x1[1] + x3[1])
    t3 = (x1[0] - x3[0], x1[1] - x3[1])
    ya = (t1[0] + t3[1], t1[1] - t3[0])
    yb = (t1[0] - t3[1], t1[1] + t3[0])
    if inverse:
        ya, yb = yb, ya
    return [(t0[0] + t2[0], t0[1] + t2[1]), ya, (t0[0] - t2[0], t0[1] - t2[1]), yb]


def _twiddle16(z, n, inverse):
    if n == 0:
        return z
    c = float(np.cos(2 * np.pi * n / 16))
    s = float(np.sin(2 * np.pi * n / 16)) * (-1.0 if inverse else 1.0)
    re, im = z
    if n % 4 == 2:
        if c * s > 0:
            return ((re + im) * c, (im - re) * c)
        return ((re - im) * c, (im + re) * c)
    return (re * c + im * s, im * c - re * s)


def _fft16(load, store, inverse):
    a = [_radix4(load(a0), load(4 + a0), load(8 + a0), load(12 + a0), inverse) for a0 in range(4)]
    for k0 in range(4):
        x0, x1, x3 = a[0][k0], _twiddle16(a[1][k0], k0, inverse), _twiddle16(a[3][k0], 3 * k0, inverse)
        if k0 == 2:
            x2 = a[2][k0]
            ta, tb = (x0[0] + x2[1], x0[1] - x2[0]), (x0[0] - x2[1], x0[1] + x2[0])
            t0, t1 = (tb, ta) if inverse else (ta, tb)
            y = _radix4_tail(t0, t1, x1, x3, inverse)
        else:
            y = _radix4(x0, x1, _twiddle16(a[2][k0], 2 * k0, inverse), x3, inverse)
        for k1 in range(4):
            store(k0 + 4 * k1, y[k1])


def _dot(a, b):
    return jnp.dot(a, b, preferred_element_type=f32)


def _dot_nt(a, b):
    return jax.lax.dot_general(a, b, (((1,), (1,)), ((), ())), preferred_element_type=f32)


def _col_mean(acc):
    part = acc[0:8]
    for i in range(8, acc.shape[0], 8):
        part = part + acc[i:i + 8]
    return jnp.broadcast_to(jnp.sum(part, axis=0, keepdims=True) * (1.0 / D), part.shape)


class _Moments:
    def __init__(self, ways):
        self.pivot, self.count, self.sums = None, 0, [None] * ways

    def add(self, x):
        if self.pivot is None:
            self.pivot = jnp.broadcast_to(x[0:1], x.shape)
        d = x - self.pivot
        way, self.count = self.count % len(self.sums), self.count + 1
        old = self.sums[way]
        self.sums[way] = (d, d * d) if old is None else (old[0] + d, old[1] + d * d)
        return d

    def mean_rstd(self, shifted=False):
        m1, m2 = (_col_mean(jnp.concatenate(s, axis=0)) for s in zip(*self.sums))
        rstd = jax.lax.rsqrt(jnp.maximum(m2 - m1 * m1, 0.0) + EPS)
        return (m1 if shifted else self.pivot[0:8] + m1), rstd


def _rows(x, n):
    return jnp.concatenate([x] * n, axis=0)


def _cols(x, n):
    return jnp.concatenate([x] * n, axis=1)


def _gelu(x):
    k = float(np.sqrt(2 / np.pi))
    t = jnp.tanh(x * (x * x * (k * 0.044715) + k))
    hx = 0.5 * x
    return hx * t + hx


def _pack(x):
    return pltpu.bitcast(x.astype(bf16), u32)


def _unpack(x):
    return pltpu.bitcast(x, bf16)


def _lhs_operands(a11, a12, a21, a22):
    return (a11 + a22, a21 + a22, a11, a22, a11 + a12, a21 - a11, a12 - a22)


def _lhs_operands2(a):
    outer = [_lhs_operands(a[p][q], a[p][q + 2], a[p + 2][q], a[p + 2][q + 2]) for p in range(2) for q in range(2)]
    return [op for four in zip(*outer) for op in _lhs_operands(*four)]


def _strassen(product, b, add, sub, emit):
    m5 = product(4, b(1, 1))
    m2 = product(1, b(0, 0))
    m3 = product(2, sub(b(0, 1), b(1, 1)))
    emit(0, 1, add(m3, m5))
    c22 = sub(m3, m2)
    m4 = product(3, sub(b(1, 0), b(0, 0)))
    emit(1, 0, add(m2, m4))
    c11 = sub(m4, m5)
    m1 = product(0, add(b(0, 0), b(1, 1)))
    c11, c22 = add(c11, m1), add(c22, m1)
    emit(0, 0, add(c11, product(6, add(b(1, 0), b(1, 1)))))
    emit(1, 1, add(c22, product(5, add(b(0, 0), b(0, 1)))))


def _strassen2(lhs, rhs, emit, after=None):
    quads = [(p, q) for p in range(2) for q in range(2)]
    order = iter(range(49))

    def add(x, y):
        return x.astype(f32) + y.astype(f32)

    def sub(x, y):
        return x.astype(f32) - y.astype(f32)

    def inner(i, b):
        out = {}

        def product(k, w):
            m = _dot(lhs(7 * i + k), w.astype(bf16))
            if after is not None:
                after(next(order), m)
            return m

        _strassen(product, lambda p, q: b[p, q], add, sub,
                  lambda p, q, value: out.__setitem__((p, q), value))
        return out

    _strassen(inner, lambda p, q: {pq: rhs(2 * p + pq[0], 2 * q + pq[1]) for pq in quads},
              lambda x, y: {pq: add(x[pq], y[pq]) for pq in quads},
              lambda x, y: {pq: sub(x[pq], y[pq]) for pq in quads},
              lambda p, q, value: [emit(2 * p + pq[0], 2 * q + pq[1], value[pq]) for pq in value])


def _interleave(main, side):
    done = 0
    for i, job in enumerate(main):
        job()
        upto = (i + 1) * len(side) // len(main)
        for s in side[done:upto]:
            s()
        done = upto


XC = 8
RU = 4
XT = NT // XC
QD = D // 4
N1 = F // 4 // L
N2 = S // 4 // L
PACE = (2, 3, 4, 5, 6, 10, 11, 12, 13)
M_A, M_B, M_C = 2 * D // L, -(-5 * D // L), 6 * D // L


def _kernel(xT_hbm, wr_hbm, wi_hbm, w1_hbm, b1_hbm, w2_hbm, b2_hbm, c_hbm, wm_hbm, dm_hbm, o_hbm,
            x_v, w_v, w1_v, w2_v, wm_v, dm_v, dm_f, mod_v, t_v, wpa_v, wpb_v, ha_v,
            hb_v, ga_v, gb_v, ta_v, tb_v, h2_v, x1_v, a1_v, a2_v, o_v, b1_v, b2_v, c_v, b1_f, b2_f, mr_v, st_v,
            sem, sem_x, sem_w1, sem_w2):
    def lanes(i, n=L):
        return pl.ds(pl.multiple_of(i * n, n), n)

    def copy(src, dst, i):
        return pltpu.make_async_copy(src, dst, sem.at[i])

    def cp_wm(t0, t1, i):
        return copy(wm_hbm.at[:, t0 * L:t1 * L], wm_v.at[:, t0 * L:t1 * L], i)

    cp_c = copy(c_hbm, c_v, 0)
    cp_df, cp_di = copy(dm_hbm.at[0:5], dm_v.at[0:5], 1), copy(dm_hbm.at[5:10], dm_v.at[5:10], 11)
    cp_wma, cp_wmb = cp_wm(0, M_A, 2), cp_wm(M_A, M_C, 3)
    cp_wa = [copy(w.at[0:RA], w_v.at[z, 0:RA], 5 + z) for z, w in enumerate((wr_hbm, wi_hbm))]
    cp_wb = [copy(w.at[RA:DF], w_v.at[z, RA:DF], 7 + z) for z, w in enumerate((wr_hbm, wi_hbm))]
    cp_b1, cp_b2 = copy(b1_hbm, b1_v, 9), copy(b2_hbm, b2_v, 10)

    def cp_x(a):
        return pltpu.make_async_copy(xT_hbm.at[:, lanes(a)], x_v.at[a], sem_x.at[a // XT])

    def cp_w1(j, q):
        return pltpu.make_async_copy(w1_hbm.at[:, lanes(j + q * N1)], w1_v.at[j, q], sem_w1.at[j])

    def cp_w2(a):
        return pltpu.make_async_copy(w2_hbm.at[:, lanes(a)], w2_v.at[a], sem_w2.at[a % N2])

    def cp_o(a, h):
        rows = slice(h * D // 2, (h + 1) * D // 2)
        return pltpu.make_async_copy(o_v.at[a, rows], o_hbm.at[rows, lanes(a)], sem.at[4])

    def loop(n, body):
        jax.lax.fori_loop(0, n, lambda i, c: (body(i), c)[1], 0)

    def start_in_order(copies):
        def body(i, total):
            for k, cp in enumerate(copies):
                pl.when(i == k)(cp.start)
            return total + i

        return jax.lax.fori_loop(0, len(copies), body, 0)

    start_in_order([cp_c, cp_wma] + [cp_x(a) for a in range(XT)] + [cp_df])
    loop(NT - XT, lambda a: cp_x(a + XT).start())
    total = start_in_order(cp_wa + cp_wb + [cp_wmb, cp_di, cp_b1, cp_b2])
    yes = total > 0
    always = jax.lax.broadcasted_iota(jnp.int32, (8, L), 0) < total

    row = jax.lax.broadcasted_iota(jnp.int32, (L, L), 0)
    lane = jax.lax.broadcasted_iota(jnp.int32, (L, L), 1)
    ang = ((row * (8 * (lane & 15) + (lane >> 4))) & 127).astype(f32) * float(2 * np.pi / L)
    step = row.astype(f32) * float(2 * np.pi / S)
    ec, es = jnp.cos(step), jnp.sin(step)
    tc, ts = jnp.cos(ang), jnp.sin(ang)
    for k1 in range(NT):
        for n, m in enumerate((tc, tc - ts, -ts - tc)):
            m = _pack(m)
            t_v[k1, n] = pltpu.roll(m, k1, 1) if k1 else m
        tc, ts = tc * ec - ts * es, ts * ec + tc * es

    cp_c.wait()
    cf = c_v[...].astype(f32)
    sc = jnp.broadcast_to(cf * jax.nn.sigmoid(cf), (8, D))

    def mod_row(t):
        m = _dot(sc, wm_v[:, t * L:(t + 1) * L])
        mr_v[t] = m
        return m

    def mod_col(t):
        col = _rows(mr_v[t], L // 8).T
        for r0, r1 in ((0, L // 2), (L // 2, L)):
            one = (t * L + r0) // D in (1, 4)
            mod_v[t * L + r0:t * L + r1, :] = col[r0:r1] + 1.0 if one else col[r0:r1]

    with jax.named_scope("w_wma"):
        cp_wma.wait()
    with jax.named_scope("mod_a"):
        for t in range(M_A):
            mod_row(t)
            mod_col(t)

    def channel_dft(i):
        for t in range(XT):
            a = i * XT + t
            for g in range(4):
                o = _dot(dm_f[g], ta_v[t, 128 * g:128 * g + 128, :])
                for z in range(2):
                    ha_v[a, z, 32 * g:32 * g + 32, :] = o[64 * z:64 * z + 32]
                    hb_v[a, z, 32 * g:32 * g + 32, :] = o[64 * z + 32:64 * z + 64]
            o = _dot(dm_f[4, 0:72, 0:64], ta_v[t, 512:D, :])
            ha_v[a, 0, 128:RA, :] = o[0:16]
            hb_v[a, 0, 128:RB, :] = o[16:40]
            ha_v[a, 1, 128:RA, :] = o[40:56]
            hb_v[a, 1, 128:RA, :] = o[56:72]
            hb_v[a, 1, RA:RB, :] = jnp.zeros((8, L), f32)

    def ln_stats(i):
        for t in range(XT):
            a = i * XT + t
            moments = _Moments(1)
            for r in range(0, D, 32):
                moments.add(x_v[a, r:r + 32, :].astype(f32))
            st_v[t, 0], st_v[t, 1] = moments.mean_rstd()

    def ln_radix9(i):
        for r in range(0, 64, 8):
            for t in range(XT):
                mean, rstd = st_v[t, 0], st_v[t, 1]
                hb = [(x_v[i * XT + t, q:q + 8, :].astype(f32) - mean) * rstd * mod_v[D + q:D + q + 8, :]
                      + mod_v[q:q + 8, :] for q in range(r, D, 64)]
                p = [hb[j] + hb[9 - j] for j in range(1, 5)]
                m = [hb[j] - hb[9 - j] for j in range(1, 5)]
                ev, od = _radix9(hb[0], p[0], p[1], p[2], p[3], m[0], m[1], m[2], m[3])
                for g in range(4):
                    ta_v[t, 128 * g + 2 * r:128 * g + 2 * r + 8, :] = ev[g + 1]
                    ta_v[t, 128 * g + 2 * r + 8:128 * g + 2 * r + 16, :] = od[g]
                ta_v[t, 512 + r:512 + r + 8, :] = ev[0]

    def wait_x(i):
        for t in range(XT):
            cp_x(i * XT + t).wait()

    def fwd_step(i):
        wait_x(i)
        channel_dft(i - 1)
        ln_stats(i)
        ln_radix9(i)
        for q in range(4):
            cp_w1(i, q).start()

    with jax.named_scope("fwd"):
        wait_x(0)
        ln_stats(0)
        ln_radix9(0)
        cp_df.wait()
        dm_f[0:5] = dm_v[0:5].astype(f32)
        for q in range(4):
            cp_w1(0, q).start()
        loop(XC - 1, lambda i: fwd_step(i + 1))
        channel_dft(XC - 1)
        for q in range(4):
            cp_w1(XC, q).start()

    def radix16(src, dst, p, inverse, tie=None):
        rows = slice(8 * p, 8 * p + 8) if isinstance(p, int) else lanes(p, 8)

        def load(a):
            x = (src[a, 0, rows, :], src[a, 1, rows, :])
            if tie is not None and a < 4:
                x = (jnp.where(always, x[0], tie[32 * a:32 * a + 8]), jnp.where(always, x[1], tie[32 * a + 16:32 * a + 24]))
            return x

        def store(k, y):
            dst[k, 0, rows, :] = y[0]
            dst[k, 1, rows, :] = y[1]

        _fft16(load, store, inverse)

    def dft128(src, dst, k):
        gr, gi = src[k, 0], src[k, 1]
        p1 = _dot(gr + gi, _unpack(t_v[k, 0]))
        xr = p1 - _dot(gi, _unpack(t_v[k, 1]))
        dst[k, 0] = xr
        dst[k, 1] = p1 + _dot(gr, _unpack(t_v[k, 2]))
        return xr

    lane8 = jax.lax.broadcasted_iota(jnp.int32, (8, L), 1)

    def permute(tiles, dst, z, rows):
        rot = [tiles[0]] + [pltpu.roll(tiles[j], j, 1) for j in range(1, NT)]
        cur = [rot[-i % NT] for i in range(NT)]
        for b in range(4):
            mask = ((lane8 >> b) & 1) == 1
            cur = [jnp.where(mask, cur[(i - (1 << b)) % NT], cur[i]) for i in range(NT)]
        for k in range(NT):
            dst[k, z, rows, :] = cur[k]

    def permute_rows(dst, z, r0, p):
        permute([pltpu.bitcast(w_v[z, r0 + 16 * p:r0 + 16 * p + 16, j * L:(j + 1) * L], u32) for j in range(NT)],
                dst, z, slice(8 * p, 8 * p + 8))

    def permute_nyquist(z):
        nyq = w_v[z, DF - 1:DF, :].astype(f32)
        permute([pltpu.bitcast(jnp.broadcast_to(nyq[:, j * L:(j + 1) * L], (8, L)), u32) for j in range(NT)],
                wpb_v, z, slice(72, 80))

    def idft128(src, wp, dst, k):
        def filt(z):
            blocks = []
            for rho in _ORDER:
                w = wp[k, z, pl.ds(rho // 2, 8, stride=9), :]
                blocks.append(pltpu.bitcast((w & u32(0xFFFF0000)) if rho % 2 else (w << 16), f32))
            if wp is wpb_v:
                blocks.append(pltpu.bitcast(wp[k, z, 72:80, :], f32))
            return jnp.concatenate(blocks, axis=0)

        xr, xi, wr, wi = src[k, 0], src[k, 1], filt(0), filt(1)
        yr, yi = xr * wr - xi * wi, xr * wi + xi * wr
        q1 = _dot_nt(yr + yi, _unpack(t_v[k, 0]))
        zr = q1 + _dot_nt(yi, _unpack(t_v[k, 2]))
        dst[k, 0] = zr
        dst[k, 1] = q1 - _dot_nt(yr, _unpack(t_v[k, 1]))
        return zr

    def paced_radix16(jobs, src, dst, n, inverse):
        for p in range(n - len(jobs)):
            radix16(src, dst, p, inverse)
        for p, job in enumerate(jobs):
            radix16(src, dst, n - len(jobs) + p, inverse, job())

    with jax.named_scope("s1"):
        loop(6, lambda i: [radix16(ha_v, ga_v, 3 * i + t, False) for t in range(3)])
    with jax.named_scope("s2"):
        pl.when(yes)(lambda: paced_radix16([lambda k=k: dft128(ga_v, ha_v, k) for k in range(NT)],
                                           hb_v, gb_v, RB // 8, False))
    with jax.named_scope("w_wa"):
        for cp in cp_wa:
            cp.wait()
    with jax.named_scope("s3"):
        pl.when(yes)(lambda: _interleave(
            [lambda k=k: dft128(gb_v, hb_v, k) for k in range(NT)],
            [lambda z=z, p=p: permute_rows(wpa_v, z, 0, p) for z in range(2) for p in range(9)]))
    with jax.named_scope("w_wb"):
        for cp in cp_wb:
            cp.wait()
    with jax.named_scope("s4"):
        pl.when(yes)(lambda: _interleave(
            [lambda k=k: idft128(ha_v, wpa_v, ga_v, k) for k in range(NT)],
            [lambda z=z, p=p: permute_rows(wpb_v, z, RA, p) for z in range(2) for p in range(9)]
            + [lambda z=z: permute_nyquist(z) for z in range(2)]))
    with jax.named_scope("s5"):
        pl.when(yes)(lambda: paced_radix16([lambda k=k: idft128(hb_v, wpb_v, gb_v, k) for k in range(NT)],
                                           ga_v, ha_v, RA // 8, True))
    with jax.named_scope("w_wmb"):
        cp_wmb.wait()
    with jax.named_scope("s6"):
        pl.when(yes)(lambda: paced_radix16([lambda t=t: _rows(mod_row(t), 16) for t in range(M_A, M_C)],
                                           gb_v, hb_v, RB // 8, True))
    cp_di.wait()
    dm_f[5:10] = dm_v[5:10].astype(f32)
    cp_b1.wait()
    cp_b2.wait()
    b1_f[...] = b1_v[...].astype(f32)
    b2_f[...] = b2_v[...].astype(f32)

    def pair_tiles(n):
        first = n // 2 + (n % 2) * (NT // 2)
        return first, first + NT // 4

    def channel_idft(n, ties=None):
        for t, a in enumerate(pair_tiles(n)):
            for g in (4, 0, 1, 2, 3):
                if g == 4:
                    rhs = [ha_v[a, 0, 128:RA, :], hb_v[a, 0, 128:RB, :], ha_v[a, 1, 128:RA, :], hb_v[a, 1, 128:RA, :]]
                else:
                    rhs = [ref[a, z, 32 * g:32 * g + 32, :] for z in range(2) for ref in (ha_v, hb_v)]
                rhs = jnp.concatenate(rhs, axis=0)
                if ties is not None:
                    rhs = jnp.concatenate([rhs[:-8], jnp.where(always, rhs[-8:], next(ties))], axis=0)
                if g == 4:
                    tb_v[t, 512:D, :] = _dot(dm_f[9, 0:64, 0:72], rhs)
                else:
                    tb_v[t, 128 * g:128 * g + 128, :] = _dot(dm_f[5 + g], rhs)

    def inv_pair(n):
        tiles, stats, ties = pair_tiles(n), [], []
        for t, a in enumerate(tiles):
            moments = _Moments(2)
            for r in range(0, 64, 8):
                al = [tb_v[t, 128 * g + 2 * r:128 * g + 2 * r + 8, :] for g in range(4)]
                be = [tb_v[t, 128 * g + 2 * r + 8:128 * g + 2 * r + 16, :] for g in range(4)]
                ev, od = _radix9(tb_v[t, 512 + r:512 + r + 8, :], *al, *be)
                y = [ev[0]] + [ev[j + 1] - od[j] for j in range(4)] + [ev[j + 1] + od[j] for j in (3, 2, 1, 0)]
                for j in range(9):
                    q = 64 * j + r
                    x1 = x_v[a, q:q + 8, :].astype(f32) + mod_v[2 * D + q:2 * D + q + 8, :] * y[j]
                    x1_v[a, q:q + 8, :] = x1
                    moments.add(x1)
                ties.append(ev[0])
            stats.append(moments.mean_rstd())
        channel_idft(jnp.minimum(n + 1, NT // 2 - 1), iter(ties[0:10]))
        moments = [_Moments(2), _Moments(2)]
        for q in range(0, D, 8):
            for t, (mean, rstd) in enumerate(stats):
                z = ((x1_v[tiles[t], q:q + 8, :] - mean) * rstd * mod_v[4 * D + q:4 * D + q + 8, :]
                     + mod_v[3 * D + q:3 * D + q + 8, :])
                h2_v[2 * (n % 2) + t, q:q + 8, :] = moments[t].add(z)
        for t in range(2):
            st_v[2 * (n % 2) + t, 0], st_v[2 * (n % 2) + t, 1] = moments[t].mean_rstd(shifted=True)

    def left_operands(dst, slot, r, prep):
        blocks = [[prep(p, q, h2_v[q, pl.ds(QD * p + r, 16), :]) for q in range(4)] for p in range(4)]
        for n, op in enumerate(_lhs_operands2(blocks)):
            dst[slot, n, pl.ds(r, 16), :] = op.astype(bf16)

    def paced(tie):
        return lambda p, q, g: jnp.where(_rows(always, 2), g, tie) if p // 2 == q // 2 else g

    def inv_body(i):
        for q in range(4):
            cp_w2(i + q * N2).start()
        loop(2, lambda half: inv_pair(2 * i + half))
        for r in range(0, QD, 16):
            left_operands(a1_v, i, r, lambda p, q, z: (z - _rows(st_v[q, 0], 2)) * _rows(st_v[q, 1], 2))

    with jax.named_scope("inv"):
        channel_idft(0)
        for t in range(M_A, M_C):
            mod_col(t)
        loop(NT // 4, inv_body)

    def mm1_body(j):

        def emit(p, q, u):
            h2_v[q, p * QD:(p + 1) * QD, :] = _gelu(u + b1_f[pl.ds(j + q * N1, 1), :])

        def after(n, m):
            if n in PACE:
                left_operands(a2_v, (j + N1 - 1) % N1, 16 * PACE.index(n), paced(m[0:16]))

        _strassen2(lambda n: jnp.concatenate([a1_v[k, n] for k in range(N2)], axis=1),
                   lambda p, q: w1_v[j, q, p * S // 4:(p + 1) * S // 4, :], emit, after)

    with jax.named_scope("mm1"):
        loop(N1 // 3, lambda i: [[cp_w1(3 * i + u, q).wait() for u in range(3) for q in range(4)], [mm1_body(3 * i + u) for u in range(3)]])

    for r in range(0, QD, 16):
        left_operands(a2_v, N1 - 1, r, lambda p, q, g: g)

    def mm2_body(j):
        for q in range(4):
            cp_w2(j + q * N2).wait()
        done = set()

        def emit(p, q, y):
            a, rows = j + q * N2, slice(p * QD, (p + 1) * QD)
            gate = mod_v[5 * D + rows.start:5 * D + rows.stop, :]
            o_v[a, rows, :] = (x1_v[a, rows, :] + gate * (y + b2_f[pl.ds(a, 1), :])).astype(bf16)
            done.add((p, q))
            if (p ^ 1, q) in done:
                cp_o(a, p // 2).start()

        _strassen2(lambda n: jnp.concatenate([a2_v[k, n] for k in range(N1)], axis=1),
                   lambda p, q: w2_v[j + q * N2, p * F // 4:(p + 1) * F // 4, :], emit)

    with jax.named_scope("mm2"):
        loop(N2, mm2_body)
    with jax.named_scope("w_out"):
        loop(NT, lambda a: [cp_o(a, h).wait() for h in range(2)])


@jax.jit
def pallas_adaLN_cond__spectral_gfnet__mixer_token_mlp__prompt_kernel(
    A_x: jax.Array,
    A_w_r: jax.Array,
    A_w_i: jax.Array,
    B_x: jax.Array,
    B_w1: jax.Array,
    B_b1: jax.Array,
    B_w2: jax.Array,
    B_b2: jax.Array,
    c: jax.Array,
    w_mod: jax.Array,
):
    del B_x
    outT = pl.pallas_call(
        _kernel,
        out_shape=jax.ShapeDtypeStruct((D, S), bf16),
        in_specs=[pl.BlockSpec(memory_space=pl.ANY)] * 10,
        out_specs=pl.BlockSpec(memory_space=pl.ANY),
        scratch_shapes=[
            pltpu.VMEM((NT, D, L), bf16),
            pltpu.VMEM((2, DF, S), bf16),
            pltpu.VMEM((N1, 4, S, L), bf16),
            pltpu.VMEM((NT, F, L), bf16),
            pltpu.VMEM((D, 6 * D), bf16),
            pltpu.VMEM((10, L, L), bf16),
            pltpu.VMEM((10, L, L), f32),
            pltpu.VMEM((6 * D, L), f32),
            pltpu.VMEM((NT, 3, L // 2, L), u32),
            pltpu.VMEM((NT, 2, 72, L), u32),
            pltpu.VMEM((NT, 2, 80, L), u32),
            pltpu.VMEM((NT, 2, RA, L), f32),
            pltpu.VMEM((NT, 2, RB, L), f32),
            pltpu.VMEM((NT, 2, RA, L), f32),
            pltpu.VMEM((NT, 2, RB, L), f32),
            pltpu.VMEM((2, D, L), f32),
            pltpu.VMEM((2, D, L), f32),
            pltpu.VMEM((4, D, L), f32),
            pltpu.VMEM((NT, D, L), f32),
            pltpu.VMEM((N2, 49, QD, L), bf16),
            pltpu.VMEM((N1, 49, QD, L), bf16),
            pltpu.VMEM((NT, D, L), bf16),
            pltpu.VMEM((F // L, L), bf16),
            pltpu.VMEM((NT, L), bf16),
            pltpu.VMEM((1, D), bf16),
            pltpu.VMEM((F // L, L), f32),
            pltpu.VMEM((NT, L), f32),
            pltpu.VMEM((M_C, 8, L), f32),
            pltpu.VMEM((4, 2, 8, L), f32),
            pltpu.SemaphoreType.DMA((12,)),
            pltpu.SemaphoreType.DMA((XC,)),
            pltpu.SemaphoreType.DMA((N1,)),
            pltpu.SemaphoreType.DMA((N2,)),
        ],
        compiler_params=pltpu.CompilerParams(vmem_limit_bytes=120 * 1024 * 1024),
        name="adaln_gfnet_token_mlp",
    )(A_x[0].T, A_w_r.T, A_w_i.T, B_w1, B_b1.reshape(F // L, L), B_w2, B_b2.reshape(NT, L), c, w_mod,
      _DMAT)
    return outT.T[None]
```

```python
import numpy as np

import jax
import jax.numpy as jnp
import jax.experimental.pallas as pl
import jax.experimental.pallas.tpu as pltpu

S, D, F = 2048, 576, 4608
DF = D // 2 + 1
L = 128
NT = S // L
XT = 2
RA, RB = 144, 152
QD = D // 4
N1 = F // 4 // L
N2 = S // 4 // L
M_A, M_B, M_C = 2 * D // L, 15, 6 * D // L
PACE = (1, 2, 3, 4, 5, 9, 10, 11, 12)
EPS = 1e-5
f32, bf16, u32 = jnp.float32, jnp.bfloat16, jnp.uint32

_ORDER = (1, 10, 8, 17, 2, 11, 7, 16, 3, 12, 6, 15, 4, 13, 5, 14, 0, 9)
_S3 = float(np.sin(2 * np.pi / 3))
_C1, _C2, _C4 = (float(np.cos(2 * np.pi * k / 9)) for k in (1, 2, 4))
_S1, _S2, _S4 = (float(np.sin(2 * np.pi * k / 9)) / _S3 for k in (1, 2, 4))


def _channel_dft_matrices():
    dp = np.arange(64)
    ca = (dp // 8) * 16 + dp % 8
    cb = ca + 8
    fw = np.zeros((5, L, L))
    iv = np.zeros((5, L, L))
    for h in range(2):
        for m in range(8):
            for g in range(4):
                for q in range(4):
                    rho = _ORDER[4 * g + q]
                    sig = _S3 if rho % 9 == g + 1 else -_S3
                    phi = 2 * np.pi * dp * (18 * (8 * h + m) + rho) / D
                    re = 32 * h + 8 * q + m
                    im = 64 + re
                    c = 2.0 / (D * S)
                    fw[g, re, ca], fw[g, re, cb] = np.cos(phi), -sig * np.sin(phi)
                    fw[g, im, ca], fw[g, im, cb] = -np.sin(phi), -sig * np.cos(phi)
                    iv[g, ca, re], iv[g, ca, im] = c * np.cos(phi), -c * np.sin(phi)
                    iv[g, cb, re], iv[g, cb, im] = sig * c * np.sin(phi), sig * c * np.cos(phi)
            for q in range(2):
                kd = 18 * (8 * h + m) + _ORDER[16 + q]
                phi = 2 * np.pi * dp * kd / D
                re = 16 * h + 8 * q + m
                im = 40 + re
                c = (1.0 if kd == 0 else 2.0) / (D * S)
                fw[4, re, :64], fw[4, im, :64] = np.cos(phi), -np.sin(phi)
                iv[4, :64, re], iv[4, :64, im] = c * np.cos(phi), -c * np.sin(phi)
    fw[4, 32, :64] = np.cos(np.pi * dp)
    iv[4, :64, 32] = np.cos(np.pi * dp) / (D * S)
    return np.concatenate([fw, iv], 0).astype(np.float32).astype(bf16)


_DMAT = _channel_dft_matrices()


def _radix9(h0, p1, p2, p3, p4, m1, m2, m3, m4):
    e = p1 + p2 + p4
    f = h0 + p3
    base = h0 - 0.5 * p3
    a, b = p1 - p4, p2 - p4
    r1, r2 = _C1 * a + _C2 * b, _C2 * a + _C4 * b
    u, v = m1 + m2, m2 + m4
    i1, i2 = _S1 * u + _S4 * v, _S2 * u - _S1 * v
    return ((f + e, base + r1, base + r2, f - 0.5 * e, base - (r1 + r2)),
            (i1 + m3, i2 - m3, m1 - m2 + m4, (i2 - i1) + m3))


def _radix4(x0, x1, x2, x3, inverse):
    t0 = (x0[0] + x2[0], x0[1] + x2[1])
    t1 = (x0[0] - x2[0], x0[1] - x2[1])
    return _radix4_tail(t0, t1, x1, x3, inverse)


def _radix4_tail(t0, t1, x1, x3, inverse):
    t2 = (x1[0] + x3[0], x1[1] + x3[1])
    t3 = (x1[0] - x3[0], x1[1] - x3[1])
    ya = (t1[0] + t3[1], t1[1] - t3[0])
    yb = (t1[0] - t3[1], t1[1] + t3[0])
    if inverse:
        ya, yb = yb, ya
    return [(t0[0] + t2[0], t0[1] + t2[1]), ya, (t0[0] - t2[0], t0[1] - t2[1]), yb]


def _twiddle16(z, n, inverse):
    if n == 0:
        return z
    c = float(np.cos(2 * np.pi * n / 16))
    s = float(np.sin(2 * np.pi * n / 16)) * (-1.0 if inverse else 1.0)
    re, im = z
    if n % 4 == 2:
        if c * s > 0:
            return ((re + im) * c, (im - re) * c)
        return ((re - im) * c, (im + re) * c)
    return (re * c + im * s, im * c - re * s)


def _fft16(load, store, inverse):
    a = [_radix4(load(a0), load(4 + a0), load(8 + a0), load(12 + a0), inverse) for a0 in range(4)]
    for k0 in range(4):
        x0, x1, x3 = a[0][k0], _twiddle16(a[1][k0], k0, inverse), _twiddle16(a[3][k0], 3 * k0, inverse)
        if k0 == 2:
            x2 = a[2][k0]
            ta, tb = (x0[0] + x2[1], x0[1] - x2[0]), (x0[0] - x2[1], x0[1] + x2[0])
            t0, t1 = (tb, ta) if inverse else (ta, tb)
            y = _radix4_tail(t0, t1, x1, x3, inverse)
        else:
            y = _radix4(x0, x1, _twiddle16(a[2][k0], 2 * k0, inverse), x3, inverse)
        for k1 in range(4):
            store(k0 + 4 * k1, y[k1])


def _dot(a, b):
    return jnp.dot(a, b, preferred_element_type=f32)


def _dot_nt(a, b):
    return jax.lax.dot_general(a, b, (((1,), (1,)), ((), ())), preferred_element_type=f32)


def _rows(x, n):
    return jnp.concatenate([x] * n, axis=0)


class _Moments:
    def __init__(self, ways):
        self.pivot, self.count, self.sums = None, 0, [None] * ways

    def add(self, x):
        if self.pivot is None:
            self.pivot = jnp.broadcast_to(x[0:1], x.shape)
        d = x - self.pivot
        way, self.count = self.count % len(self.sums), self.count + 1
        old = self.sums[way]
        self.sums[way] = (d, d * d) if old is None else (old[0] + d, old[1] + d * d)
        return d

    def mean_rstd(self, shifted=False):
        def mean(parts):
            parts = jnp.concatenate(parts, axis=0)
            total = parts[0:8]
            for i in range(8, parts.shape[0], 8):
                total = total + parts[i:i + 8]
            return jnp.broadcast_to(jnp.sum(total, axis=0, keepdims=True) * (1.0 / D), total.shape)

        m1, m2 = (mean(parts) for parts in zip(*self.sums))
        rstd = jax.lax.rsqrt(jnp.maximum(m2 - m1 * m1, 0.0) + EPS)
        return (m1 if shifted else self.pivot[0:8] + m1), rstd


def _gelu(x):
    k = float(np.sqrt(2 / np.pi))
    half = 0.5 * x
    return half * jnp.tanh(x * (x * x * (k * 0.044715) + k)) + half


def _lhs_operands(a11, a12, a21, a22):
    return (a11 + a22, a21 + a22, a11, a22, a11 + a12, a21 - a11, a12 - a22)


def _lhs_operands2(a):
    outer = [_lhs_operands(a[p][q], a[p][q + 2], a[p + 2][q], a[p + 2][q + 2]) for p in range(2) for q in range(2)]
    return [op for four in zip(*outer) for op in _lhs_operands(*four)]


def _strassen(product, b, add, sub, emit):
    m5 = product(4, b(1, 1))
    m2 = product(1, b(0, 0))
    m3 = product(2, sub(b(0, 1), b(1, 1)))
    emit(0, 1, add(m3, m5))
    c22 = sub(m3, m2)
    m4 = product(3, sub(b(1, 0), b(0, 0)))
    emit(1, 0, add(m2, m4))
    c11 = sub(m4, m5)
    m1 = product(0, add(b(0, 0), b(1, 1)))
    c11, c22 = add(c11, m1), add(c22, m1)
    emit(0, 0, add(c11, product(6, add(b(1, 0), b(1, 1)))))
    emit(1, 1, add(c22, product(5, add(b(0, 0), b(0, 1)))))


def _strassen2(lhs, rhs, emit, after=None):
    quads = [(p, q) for p in range(2) for q in range(2)]
    order = iter(range(49))

    def add(x, y):
        return x.astype(f32) + y.astype(f32)

    def sub(x, y):
        return x.astype(f32) - y.astype(f32)

    def inner(i, b):
        out = {}

        def product(k, w):
            m = _dot(lhs(7 * i + k), w.astype(bf16))
            if after is not None:
                after(next(order), m)
            return m

        _strassen(product, lambda p, q: b[p, q], add, sub, lambda p, q, value: out.update({(p, q): value}))
        return out

    _strassen(inner, lambda p, q: {pq: rhs(2 * p + pq[0], 2 * q + pq[1]) for pq in quads},
              lambda x, y: {pq: add(x[pq], y[pq]) for pq in quads},
              lambda x, y: {pq: sub(x[pq], y[pq]) for pq in quads},
              lambda p, q, value: [emit(2 * p + pq[0], 2 * q + pq[1], value[pq]) for pq in value])


def _loop(n, body):
    jax.lax.fori_loop(0, n, lambda i, c: (body(i), c)[1], 0)


def _span(i, n):
    return pl.ds(pl.multiple_of(i * n, n), n)


def _kernel(xT_hbm, wr_hbm, wi_hbm, w1_hbm, b1_hbm, w2_hbm, b2_hbm, c_hbm, wm_hbm, dm_hbm, o_hbm,
            x_v, w_v, w1_v, w2_v, wm_v, dm_v, dm_f, mod_v, t_v, wpa_v, wpb_v, ha_v, hb_v, ga_v, gb_v,
            ta_v, tb_v, h2_v, x1_v, a1_v, a2_v, o_v, b1_v, b2_v, c_v, b1_f, b2_f, mr_v, st_v,
            sem, sem_x, sem_w1, sem_w2):
    def copy(src, dst, i):
        return pltpu.make_async_copy(src, dst, sem.at[i])

    cp_c = copy(c_hbm, c_v, 0)
    cp_df, cp_di = copy(dm_hbm.at[0:5], dm_v.at[0:5], 1), copy(dm_hbm.at[5:10], dm_v.at[5:10], 2)
    cp_wma = copy(wm_hbm.at[:, 0:M_A * L], wm_v.at[:, 0:M_A * L], 3)
    cp_wmb = copy(wm_hbm.at[:, M_A * L:M_C * L], wm_v.at[:, M_A * L:M_C * L], 4)
    cp_wa = [copy(w.at[0:RA], w_v.at[z, 0:RA], 5) for z, w in enumerate((wr_hbm, wi_hbm))]
    cp_wb = [copy(w.at[RA:DF], w_v.at[z, RA:DF], 6) for z, w in enumerate((wr_hbm, wi_hbm))]
    cp_b1, cp_b2 = copy(b1_hbm, b1_v, 7), copy(b2_hbm, b2_v, 8)

    def cp_x(a):
        return pltpu.make_async_copy(xT_hbm.at[:, _span(a, L)], x_v.at[a], sem_x.at[a // XT])

    def cp_w1(j, q):
        return pltpu.make_async_copy(w1_hbm.at[:, _span(j + q * N1, L)], w1_v.at[j, q], sem_w1.at[j])

    def cp_w2(j, q):
        return pltpu.make_async_copy(w2_hbm.at[:, _span(j + q * N2, L)], w2_v.at[j + q * N2], sem_w2.at[j])

    def cp_o(a, h):
        rows = slice(h * D // 2, (h + 1) * D // 2)
        return copy(o_v.at[a, rows], o_hbm.at[rows, _span(a, L)], 9)

    def start_in_order(copies):
        def body(i, total):
            for k, cp in enumerate(copies):
                pl.when(i == k)(cp.start)
            return total + i

        return jax.lax.fori_loop(0, len(copies), body, 0)

    start_in_order([cp_c, cp_wma] + [cp_x(a) for a in range(XT)] + [cp_df])
    _loop(NT - XT, lambda a: cp_x(a + XT).start())
    total = start_in_order(cp_wa + cp_wb + [cp_wmb, cp_di, cp_b1, cp_b2])

    stage = pl.when(total > 0)
    always = jax.lax.broadcasted_iota(jnp.int32, (8, L), 0) < total

    def behind(x, other):
        return jnp.where(_rows(always, x.shape[0] // 8), x, other)

    row = jax.lax.broadcasted_iota(jnp.int32, (L, L), 0)
    lane = jax.lax.broadcasted_iota(jnp.int32, (L, L), 1)
    angle = ((row * (8 * (lane & 15) + (lane >> 4))) & 127).astype(f32) * float(2 * np.pi / L)
    step = row.astype(f32) * float(2 * np.pi / S)
    ec, es = jnp.cos(step), jnp.sin(step)
    tc, ts = jnp.cos(angle), jnp.sin(angle)
    for k1 in range(NT):
        for n, m in enumerate((tc, tc - ts, -ts - tc)):
            m = pltpu.bitcast(m.astype(bf16), u32)
            t_v[k1, n] = pltpu.roll(m, k1, 1) if k1 else m
        tc, ts = tc * ec - ts * es, ts * ec + tc * es

    def tmat(k, n):
        return pltpu.bitcast(t_v[k, n], bf16)

    cp_c.wait()
    cf = c_v[...].astype(f32)
    sc = jnp.broadcast_to(cf * jax.nn.sigmoid(cf), (8, D))

    def mod_row(t):
        m = _dot(sc, wm_v[:, t * L:(t + 1) * L])
        mr_v[t] = m
        return m

    def mod_col(t):
        col = _rows(mr_v[t], L // 8).T
        for r0, r1 in ((0, L // 2), (L // 2, L)):
            one = (t * L + r0) // D in (1, 4)
            mod_v[t * L + r0:t * L + r1, :] = col[r0:r1] + 1.0 if one else col[r0:r1]

    def mod(i, r, n=8):
        return mod_v[i * D + r:i * D + r + n, :]

    cp_wma.wait()
    for t in range(M_A):
        mod_row(t)
        mod_col(t)

    def wait_x(i):
        for t in range(XT):
            cp_x(i * XT + t).wait()

    def ln_radix9(i):
        stats = []
        for t in range(XT):
            moments = _Moments(1)
            for r in range(0, D, 16):
                moments.add(x_v[i * XT + t, r:r + 16, :].astype(f32))
            stats.append(moments.mean_rstd())
        for r in range(0, 64, 8):
            for t, (mean, rstd) in enumerate(stats):
                h = [(x_v[i * XT + t, q:q + 8, :].astype(f32) - mean) * rstd * mod(1, q) + mod(0, q)
                     for q in range(r, D, 64)]
                ev, od = _radix9(h[0], *[h[j] + h[9 - j] for j in range(1, 5)],
                                 *[h[j] - h[9 - j] for j in range(1, 5)])
                for g in range(4):
                    ta_v[t, L * g + 2 * r:L * g + 2 * r + 8, :] = ev[g + 1]
                    ta_v[t, L * g + 2 * r + 8:L * g + 2 * r + 16, :] = od[g]
                ta_v[t, 4 * L + r:4 * L + r + 8, :] = ev[0]

    def channel_dft(i):
        for t in range(XT):
            a = i * XT + t
            for g in range(4):
                o = _dot(dm_f[g], ta_v[t, L * g:L * (g + 1), :])
                for z in range(2):
                    ha_v[a, z, 32 * g:32 * g + 32, :] = o[64 * z:64 * z + 32]
                    hb_v[a, z, 32 * g:32 * g + 32, :] = o[64 * z + 32:64 * z + 64]
            o = _dot(dm_f[4, 0:72, 0:64], ta_v[t, 4 * L:D, :])
            ha_v[a, 0, 128:RA, :] = o[0:16]
            hb_v[a, 0, 128:RB, :] = o[16:40]
            ha_v[a, 1, 128:RA, :] = o[40:56]
            hb_v[a, 1, 128:RA, :] = o[56:72]
            hb_v[a, 1, RA:RB, :] = jnp.zeros((8, L), f32)

    def start_w1(j):
        for q in range(4):
            cp_w1(j, q).start()

    wait_x(0)
    ln_radix9(0)
    cp_df.wait()
    dm_f[0:5] = dm_v[0:5].astype(f32)
    start_w1(0)
    _loop(NT // XT - 1, lambda i: (wait_x(i + 1), channel_dft(i), ln_radix9(i + 1), start_w1(i + 1)))
    channel_dft(NT // XT - 1)
    start_w1(N1 - 1)

    def radix16(src, dst, p, inverse, other=None):
        rows = slice(8 * p, 8 * p + 8) if isinstance(p, int) else _span(p, 8)

        def load(a):
            x = (src[a, 0, rows, :], src[a, 1, rows, :])
            if other is not None and a < 4:
                x = (behind(x[0], other[32 * a:32 * a + 8]), behind(x[1], other[32 * a + 16:32 * a + 24]))
            return x

        def store(k, y):
            dst[k, 0, rows, :] = y[0]
            dst[k, 1, rows, :] = y[1]

        _fft16(load, store, inverse)

    def radix16_beside(jobs, src, dst, n, inverse):
        for p in range(n - len(jobs)):
            radix16(src, dst, p, inverse)
        for p, job in enumerate(jobs):
            radix16(src, dst, n - len(jobs) + p, inverse, job())

    def dft128(src, dst, k):
        gr, gi = src[k, 0], src[k, 1]
        p1 = _dot(gr + gi, tmat(k, 0))
        xr = p1 - _dot(gi, tmat(k, 1))
        dst[k, 0] = xr
        dst[k, 1] = p1 + _dot(gr, tmat(k, 2))
        return xr

    lane8 = jax.lax.broadcasted_iota(jnp.int32, (8, L), 1)

    def permute(tiles, dst, z, rows):
        rot = [tiles[0]] + [pltpu.roll(tiles[j], j, 1) for j in range(1, NT)]
        cur = [rot[-i % NT] for i in range(NT)]
        for b in range(4):
            mask = ((lane8 >> b) & 1) == 1
            cur = [jnp.where(mask, cur[(i - (1 << b)) % NT], cur[i]) for i in range(NT)]
        for k in range(NT):
            dst[k, z, rows, :] = cur[k]

    def permute_half(dst, r0):
        for z in range(2):
            for p in range(RA // 16):
                rows = slice(r0 + 16 * p, r0 + 16 * p + 16)
                permute([pltpu.bitcast(w_v[z, rows, j * L:(j + 1) * L], u32) for j in range(NT)],
                        dst, z, slice(8 * p, 8 * p + 8))

    def permute_nyquist():
        for z in range(2):
            nyq = w_v[z, DF - 1:DF, :].astype(f32)
            permute([pltpu.bitcast(jnp.broadcast_to(nyq[:, j * L:(j + 1) * L], (8, L)), u32) for j in range(NT)],
                    wpb_v, z, slice(RA // 2, RA // 2 + 8))

    def filter_idft128(src, wp, dst, k):
        def filt(z):
            groups = []
            for rho in _ORDER:
                w = wp[k, z, pl.ds(rho // 2, 8, stride=9), :]
                groups.append(pltpu.bitcast((w & u32(0xFFFF0000)) if rho % 2 else (w << 16), f32))
            if wp is wpb_v:
                groups.append(pltpu.bitcast(wp[k, z, RA // 2:RA // 2 + 8, :], f32))
            return jnp.concatenate(groups, axis=0)

        xr, xi, wr, wi = src[k, 0], src[k, 1], filt(0), filt(1)
        yr, yi = xr * wr - xi * wi, xr * wi + xi * wr
        q1 = _dot_nt(yr + yi, tmat(k, 0))
        zr = q1 + _dot_nt(yi, tmat(k, 2))
        dst[k, 0] = zr
        dst[k, 1] = q1 - _dot_nt(yr, tmat(k, 1))
        return zr

    _loop(RA // 24, lambda i: [radix16(ha_v, ga_v, 3 * i + t, False) for t in range(3)])

    @stage
    def _():
        radix16_beside([lambda k=k: dft128(ga_v, ha_v, k) for k in range(NT)], hb_v, gb_v, RB // 8, False)

    for cp in cp_wa + cp_wb:
        cp.wait()

    @stage
    def _():
        for k in range(NT):
            dft128(gb_v, hb_v, k)
        permute_half(wpa_v, 0)
        for k in range(NT):
            filter_idft128(ha_v, wpa_v, ga_v, k)
        permute_half(wpb_v, RA)
        permute_nyquist()

    @stage
    def _():
        radix16_beside([lambda k=k: filter_idft128(hb_v, wpb_v, gb_v, k) for k in range(NT)],
                       ga_v, ha_v, RA // 8, True)

    cp_wmb.wait()

    @stage
    def _():
        radix16_beside([lambda t=t: _rows(mod_row(t), 16) for t in reversed(range(M_A, M_C))],
                       gb_v, hb_v, RB // 8, True)
        for t in range(M_B, M_C):
            mod_col(t)

    for cp in (cp_di, cp_b1, cp_b2):
        cp.wait()
    dm_f[5:10] = dm_v[5:10].astype(f32)
    b1_f[...] = b1_v[...].astype(f32)
    b2_f[...] = b2_v[...].astype(f32)

    def pair_tiles(n):
        first = n // 2 + (n % 2) * 2 * N2
        return first, first + N2

    def channel_idft(n, others=None):
        for t, a in enumerate(pair_tiles(n)):
            for g in (4, 0, 1, 2, 3):
                if g == 4:
                    rhs = [ha_v[a, 0, 128:RA, :], hb_v[a, 0, 128:RB, :], ha_v[a, 1, 128:RA, :], hb_v[a, 1, 128:RA, :]]
                else:
                    rhs = [ref[a, z, 32 * g:32 * g + 32, :] for z in range(2) for ref in (ha_v, hb_v)]
                rhs = jnp.concatenate(rhs, axis=0)
                if others is not None:
                    rhs = jnp.concatenate([rhs[:-8], behind(rhs[-8:], next(others))], axis=0)
                if g == 4:
                    tb_v[t, 4 * L:D, :] = _dot(dm_f[9, 0:64, 0:72], rhs)
                else:
                    tb_v[t, L * g:L * (g + 1), :] = _dot(dm_f[5 + g], rhs)

    def residual_norms(n):
        tiles, stats, others = pair_tiles(n), [], []
        for t, a in enumerate(tiles):
            moments = _Moments(2)
            for r in range(0, 64, 8):
                ev, od = _radix9(tb_v[t, 4 * L + r:4 * L + r + 8, :],
                                 *[tb_v[t, L * g + 2 * r:L * g + 2 * r + 8, :] for g in range(4)],
                                 *[tb_v[t, L * g + 2 * r + 8:L * g + 2 * r + 16, :] for g in range(4)])
                y = [ev[0]] + [ev[j + 1] - od[j] for j in range(4)] + [ev[j + 1] + od[j] for j in (3, 2, 1, 0)]
                for j in range(9):
                    q = 64 * j + r
                    x1 = x_v[a, q:q + 8, :].astype(f32) + mod(2, q) * y[j]
                    x1_v[a, q:q + 8, :] = x1
                    moments.add(x1)
                others.append(ev[0])
            stats.append(moments.mean_rstd())
        channel_idft(jnp.minimum(n + 1, NT // 2 - 1), iter(others))
        moments = [_Moments(2), _Moments(2)]
        for q in range(0, D, 8):
            for t, (mean, rstd) in enumerate(stats):
                z = (x1_v[tiles[t], q:q + 8, :] - mean) * rstd * mod(4, q) + mod(3, q)
                h2_v[2 * (n % 2) + t, q:q + 8, :] = moments[t].add(z)
        for t in range(2):
            st_v[2 * (n % 2) + t, 0], st_v[2 * (n % 2) + t, 1] = moments[t].mean_rstd(shifted=True)

    def left_operands(dst, slot, r, prepare):
        blocks = [[prepare(p, q, h2_v[q, QD * p + r:QD * p + r + 16, :]) for q in range(4)] for p in range(4)]
        for n, op in enumerate(_lhs_operands2(blocks)):
            dst[slot, n, r:r + 16, :] = op.astype(bf16)

    def token_operands(i):
        for q in range(4):
            cp_w2(i, q).start()
        _loop(2, lambda half: residual_norms(2 * i + half))
        for r in range(0, QD, 16):
            left_operands(a1_v, i, r, lambda p, q, z: (z - _rows(st_v[q, 0], 2)) * _rows(st_v[q, 1], 2))

    channel_idft(0)
    for t in range(M_A, M_B):
        mod_col(t)
    _loop(N2, token_operands)

    def hidden_step(j):
        def emit(p, q, u):
            h2_v[q, p * QD:(p + 1) * QD, :] = _gelu(u + b1_f[pl.ds(j + q * N1, 1), :])

        def after(n, m):
            if n in PACE:
                left_operands(a2_v, (j + N1 - 1) % N1, 16 * PACE.index(n),
                              lambda p, q, g: behind(g, m[0:16]) if p // 2 == q // 2 else g)

        _strassen2(lambda n: jnp.concatenate([a1_v[k, n] for k in range(N2)], axis=1),
                   lambda p, q: w1_v[j, q, p * S // 4:(p + 1) * S // 4, :], emit, after)

    def hidden_steps(i):
        for u in range(3):
            for q in range(4):
                cp_w1(3 * i + u, q).wait()
        for u in range(3):
            hidden_step(3 * i + u)

    _loop(N1 // 3, hidden_steps)
    for r in range(0, QD, 16):
        left_operands(a2_v, N1 - 1, r, lambda p, q, g: g)

    def output_step(j):
        for q in range(4):
            cp_w2(j, q).wait()
        done = []

        def emit(p, q, y):
            a, rows = j + q * N2, slice(p * QD, (p + 1) * QD)
            y = y + b2_f[pl.ds(a, 1), :]
            o_v[a, rows, :] = (x1_v[a, rows, :] + mod(5, p * QD, QD) * y).astype(bf16)
            done.append((p, q))
            if (p ^ 1, q) in done:
                cp_o(a, p // 2).start()

        _strassen2(lambda n: jnp.concatenate([a2_v[k, n] for k in range(N1)], axis=1),
                   lambda p, q: w2_v[j + q * N2, p * F // 4:(p + 1) * F // 4, :], emit)

    _loop(N2, output_step)
    _loop(NT, lambda a: [cp_o(a, h).wait() for h in range(2)])


@jax.jit
def pallas_adaLN_cond__spectral_gfnet__mixer_token_mlp__prompt_kernel(
    A_x: jax.Array,
    A_w_r: jax.Array,
    A_w_i: jax.Array,
    B_x: jax.Array,
    B_w1: jax.Array,
    B_b1: jax.Array,
    B_w2: jax.Array,
    B_b2: jax.Array,
    c: jax.Array,
    w_mod: jax.Array,
):
    del B_x
    outT = pl.pallas_call(
        _kernel,
        out_shape=jax.ShapeDtypeStruct((D, S), bf16),
        in_specs=[pl.BlockSpec(memory_space=pl.ANY)] * 10,
        out_specs=pl.BlockSpec(memory_space=pl.ANY),
        scratch_shapes=[
            pltpu.VMEM((NT, D, L), bf16),
            pltpu.VMEM((2, DF, S), bf16),
            pltpu.VMEM((N1, 4, S, L), bf16),
            pltpu.VMEM((NT, F, L), bf16),
            pltpu.VMEM((D, 6 * D), bf16),
            pltpu.VMEM((10, L, L), bf16),
            pltpu.VMEM((10, L, L), f32),
            pltpu.VMEM((6 * D, L), f32),
            pltpu.VMEM((NT, 3, L // 2, L), u32),
            pltpu.VMEM((NT, 2, RA // 2, L), u32),
            pltpu.VMEM((NT, 2, RA // 2 + 8, L), u32),
            pltpu.VMEM((NT, 2, RA, L), f32),
            pltpu.VMEM((NT, 2, RB, L), f32),
            pltpu.VMEM((NT, 2, RA, L), f32),
            pltpu.VMEM((NT, 2, RB, L), f32),
            pltpu.VMEM((XT, D, L), f32),
            pltpu.VMEM((2, D, L), f32),
            pltpu.VMEM((4, D, L), f32),
            pltpu.VMEM((NT, D, L), f32),
            pltpu.VMEM((N2, 49, QD, L), bf16),
            pltpu.VMEM((N1, 49, QD, L), bf16),
            pltpu.VMEM((NT, D, L), bf16),
            pltpu.VMEM((F // L, L), bf16),
            pltpu.VMEM((NT, L), bf16),
            pltpu.VMEM((1, D), bf16),
            pltpu.VMEM((F // L, L), f32),
            pltpu.VMEM((NT, L), f32),
            pltpu.VMEM((M_C, 8, L), f32),
            pltpu.VMEM((4, 2, 8, L), f32),
            pltpu.SemaphoreType.DMA((10,)),
            pltpu.SemaphoreType.DMA((NT // XT,)),
            pltpu.SemaphoreType.DMA((N1,)),
            pltpu.SemaphoreType.DMA((N2,)),
        ],
        compiler_params=pltpu.CompilerParams(vmem_limit_bytes=120 * 1024 * 1024),
        name="adaln_gfnet_token_mlp",
    )(A_x[0].T, A_w_r.T, A_w_i.T, B_w1, B_b1.reshape(F // L, L), B_w2, B_b2.reshape(NT, L), c, w_mod, _DMAT)
    return outT.T[None]
```
